```python
import os as _os
_os.environ.setdefault("JAX_PLATFORMS", "cpu")
import jax
import jax.numpy as jnp

def _softmax(x, axis=-1):
    return jax.nn.softmax(x, axis=axis)
def _gelu(x):
    return jax.nn.gelu(x, approximate=True)
def _silu(x):
    return jax.nn.silu(x)
def _sigmoid(x):
    return jax.nn.sigmoid(x)
def _layernorm(x, axis=-1, eps=1e-5):
    m = jnp.mean(x, axis=axis, keepdims=True)
    v = jnp.var(x, axis=axis, keepdims=True)
    return (x - m) / jnp.sqrt(v + eps)
def _scatter_add(tgt, idx, src, axis=0):
    return tgt.at[idx].add(src)
def _segment_sum(src, seg, n):
    return jax.ops.segment_sum(src, seg, n)
class _Rng:
    def __init__(self, key):
        self._k = key
    def _next(self):
        self._k, sub = jax.random.split(self._k)
        return sub
    def normal(self, shape):
        return jax.random.normal(self._next(), shape, dtype=jnp.bfloat16)
    def randint(self, lo, hi, shape):
        return jax.random.randint(self._next(), shape, lo, hi, dtype=jnp.int32)
    def uniform(self, shape, lo=0.0, hi=1.0):
        return jax.random.uniform(self._next(), shape, jnp.bfloat16, lo, hi)
    def permutation(self, n):
        return jax.random.permutation(self._next(), n)


kernel_name = 'parallel_sum__sliding_block__moe_arch_mod__prompt'

def setup_inputs():
    _rng = _Rng(jax.random.key(int.from_bytes(__import__("os").urandom(4), "little")))
    _w = (lambda a: (lambda t: t.astype(jnp.bfloat16) if jnp.issubdtype(t.dtype, jnp.floating) else t)(jnp.asarray(a)))
    def _A_setup():
        B, S, D = 1, 2048, 512
        return {
            "x": _w((lambda *s: _rng.normal(s) * 0.05)(B, S, D)),
            "wqkv": _w((lambda *s: _rng.normal(s) * 0.05)(D, 3 * D)),
            "wo": _w((lambda *s: _rng.normal(s) * 0.05)(D, D)),
        }
    _A_in = _A_setup()

    def _B_setup():
        B, S, D, F, C = 1, 2048, 512, 1376, 1
        return {
            "x": _w((lambda *s: _rng.normal(s) * 0.05)(B, S, D)),
            "w_r": _w((lambda *s: _rng.normal(s) * 0.05)(D)),
            "w_gate": _w((lambda *s: _rng.normal(s) * 0.05)(D, F)),
            "w_up": _w((lambda *s: _rng.normal(s) * 0.05)(D, F)),
            "w_down": _w((lambda *s: _rng.normal(s) * 0.05)(F, D)),
        }
    _B_in = _B_setup()

    return {
        "A_x": _A_in["x"],
        "A_wqkv": _A_in["wqkv"],
        "A_wo": _A_in["wo"],
        "B_x": _B_in["x"],
        "B_w_r": _B_in["w_r"],
        "B_w_gate": _B_in["w_gate"],
        "B_w_up": _B_in["w_up"],
        "B_w_down": _B_in["w_down"],
    }

def reference(A_x, A_wqkv, A_wo, B_x, B_w_r, B_w_gate, B_w_up, B_w_down):
    def _A_ref(x, wqkv, wo):
        B, S, D = x.shape
        H = 32; Dh = D // H; W = 256
        qkv = (lambda x, *d: x.transpose(*d))((x @ wqkv).reshape(B, S, 3, H, Dh), 2, 0, 3, 1, 4)
        q, k, v = qkv[0], qkv[1], qkv[2]
        scores = jnp.einsum("bhqd,bhkd->bhqk", q, k) * (Dh ** -0.5)
        idx = jnp.arange(S)
        mask = (idx[:, None] - idx[None, :] >= 0) & (idx[:, None] - idx[None, :] < W)
        scores = jnp.where(mask[None, None], scores, -1e9)
        p = _softmax(scores, axis=-1)
        o = jnp.einsum("bhqk,bhkd->bhqd", p, v)
        return (lambda x, *d: x.transpose(*d))(o, 0, 2, 1, 3).reshape(B, S, D) @ wo

    def _B_ref(x, w_r, w_gate, w_up, w_down):
        B, S, D = x.shape
        C = 1
        r = x @ w_r
        idx = jnp.argsort(-r, axis=-1)[:, :C]
        idx_e = jnp.repeat(idx.reshape(B, C, 1), D, axis=2)
        x_sel = jnp.take_along_axis(x, idx_e, axis=1)
        g = _silu(x_sel @ w_gate)
        u = x_sel @ w_up
        y = (g * u) @ w_down
        r_sel = _sigmoid(jnp.take_along_axis(r, idx, axis=1))
        y = y * r_sel.reshape(B, C, 1)
        b_off = (jnp.arange(B) * S).reshape(B, 1)
        flat_idx = (idx + b_off).reshape(B * C)
        zero = (x * 0.0).reshape(B * S, D)
        upd = _scatter_add(zero, flat_idx, y.reshape(B * C, D), axis=0)
        return x + upd.reshape(B, S, D)

    x = A_x
    xn = _layernorm(x, axis=-1)
    return x + _A_ref(xn, A_wqkv, A_wo) + _B_ref(xn, B_w_r, B_w_gate, B_w_up, B_w_down)
```

```python
import functools, math
import numpy as np
import jax
import jax.numpy as jnp
from jax import lax
import jax.experimental.pallas as pl
import jax.experimental.pallas.tpu as pltpu

S, D, H, DH, W, F = 2048, 512, 32, 16, 256, 1376
BQ = 128
HB = BQ // 2
NB = S // BQ
BF = jnp.bfloat16
F32 = jnp.float32
I32 = jnp.int32
NT = (((1,), (1,)), ((), ()))
TN = (((0,), (0,)), ((), ()))
QSCALE = (DH ** -0.5) * math.log2(math.e)
U1 = 2
OPG = 7
MODE = 5


def _pack(v):
    return pltpu.bitcast(v.astype(BF), I32)


def _unpack(v):
    return pltpu.bitcast(v, BF)


def _layernorm_bf16(xf):
    mean = jnp.mean(xf, axis=-1, keepdims=True)
    c = xf - mean
    var = jnp.mean(c * c, axis=-1, keepdims=True)
    m = mean.astype(BF).astype(F32)
    v = var.astype(BF).astype(F32)
    d = (xf - m).astype(BF).astype(F32)
    s = jnp.sqrt((v + 1e-5).astype(BF).astype(F32)).astype(BF).astype(F32)
    return (d / s).astype(BF)


def kernel(x_hbm, wqkv_hbm, wo_hbm, wr_hbm, wgt_hbm, wut_hbm, wd_hbm, o_hbm,
           x_s, wqkv_s, wo_in, wr_s, wgt_s, wut_s, wd_s,
           xa_s, xb_s, res_s, k_s, v_s, q_s, wk_s, wt_s, wo_s, ot_s, r_s, s_s, o_s,
           sem_x, sem_w, sem_o):
    def x_copy(b):
        t0 = b * BQ if isinstance(b, int) else pl.multiple_of(b * BQ, BQ)
        src0 = min(b, NB - 1) * BQ if isinstance(b, int) else pl.multiple_of(jnp.minimum(b, NB - 1) * BQ, BQ)
        return pltpu.make_async_copy(x_hbm.at[pl.ds(src0, BQ), :], x_s.at[pl.ds(t0, BQ), :], sem_x.at[b])

    def w_copy(i):
        return pltpu.make_async_copy(wqkv_hbm.at[:, i * D:(i + 1) * D], wqkv_s.at[i], sem_w.at[i])

    c_wr = pltpu.make_async_copy(wr_hbm, wr_s, sem_w.at[3])
    c_wo = pltpu.make_async_copy(wo_hbm, wo_in, sem_w.at[4])
    c_wg = pltpu.make_async_copy(wgt_hbm, wgt_s, sem_w.at[5])
    c_wu = pltpu.make_async_copy(wut_hbm, wut_s, sem_w.at[6])
    c_wd = pltpu.make_async_copy(wd_hbm, wd_s, sem_w.at[7])

    x_copy(0).start()
    w_copy(1).start()
    w_copy(0).start()
    w_copy(2).start()
    c_wr.start()
    for b in range(1, NB + 1):
        x_copy(b).start()
    c_wo.start()
    c_wg.start()
    c_wu.start()
    c_wd.start()

    def ln_rows(b, dst, r0, n):
        t0 = b * BQ + r0 if isinstance(b, int) else pl.multiple_of(b * BQ + r0, 16)
        xf = x_s[pl.ds(t0, n), :].astype(F32)
        xn = _layernorm_bf16(xf)
        xp = pltpu.bitcast(xn, I32)
        dst[r0 // 2:(r0 + n) // 2, :] = xp
        res_s[pl.ds(t0, n), :] = xf + xn.astype(F32)
        z = xp[0:8, 0:128]
        for i in range(n // 16):
            for j in range(4):
                if i or j:
                    z = z | xp[i * 8:(i + 1) * 8, j * 128:(j + 1) * 128]
        return z

    x_copy(0).wait()
    ln_rows(0, xa_s, 0, BQ)
    w_copy(1).wait()
    wk_s[...] = pltpu.bitcast(wqkv_s[1], I32)
    w_copy(0).wait()
    wt_s[0:256, :] = pltpu.bitcast(wqkv_s[0].T, I32)
    w_copy(2).wait()
    wt_s[256:512, :] = pltpu.bitcast(wqkv_s[2].T, I32)
    c_wr.wait()
    wt_s[512:520, :] = pltpu.bitcast(jnp.broadcast_to(wr_s[...], (16, D)), I32)

    lo8 = lax.broadcasted_iota(I32, (1, 8, 128), 2) < 64

    def proj_block(b, src, dst):
        h0 = b * HB if isinstance(b, int) else pl.multiple_of(b * HB, HB)
        xn = _unpack(src[...])
        kk = jnp.dot(xn, _unpack(wk_s[...]), preferred_element_type=F32)
        for g8 in range(4):
            k_s[g8, pl.ds(h0, HB), :] = _pack(kk[:, g8 * 128:(g8 + 1) * 128])
        zero = jnp.minimum(b, 0)

        def lhs(r0, r1, z):
            first = wt_s[r0:r0 + 8, :]
            first = jnp.concatenate([first[:, 0:128] | (z & zero), first[:, 128:]], axis=1)
            return _unpack(jnp.concatenate([first, wt_s[r0 + 8:r1, :]], axis=0))

        for c in range(4):
            z = ln_rows(b + 1, dst, c * 32, 32)
            r0, r1 = c * 128, (c + 1) * 128 + (8 if c == 3 else 0)
            o = lax.dot_general(lhs(r0, r1, z), xn, NT, preferred_element_type=F32)
            if c < 2:
                qp = _pack(o * QSCALE).reshape(8, 2, 8, 128)
                qr = pltpu.roll(qp, 64, axis=3)
                q_s[b, 0, c * 8:(c + 1) * 8, 0:8, :] = jnp.where(lo8, qp[:, 0], 0)
                q_s[b, 0, c * 8:(c + 1) * 8, 8:16, :] = jnp.where(lo8, 0, qr[:, 1])
                q_s[b, 1, c * 8:(c + 1) * 8, 0:8, :] = jnp.where(lo8, qr[:, 0], 0)
                q_s[b, 1, c * 8:(c + 1) * 8, 8:16, :] = jnp.where(lo8, 0, qp[:, 1])
            else:
                v_s[b, (c - 2) * 128:(c - 1) * 128, :] = _pack(o[0:256])
                if c == 3:
                    r_s[b] = o[256:264]

    def p1(i, c):
        for j in range(U1):
            x_copy(U1 * i + j + 1).wait()
        for j in range(U1):
            proj_block(U1 * i + j, (xa_s, xb_s)[j % 2], (xa_s, xb_s)[(j + 1) % 2])
        return c
    lax.fori_loop(0, NB // U1, p1, 0)

    c_wo.wait()
    wo_s[...] = pltpu.bitcast(wo_in[...], I32)
    r = r_s[...].astype(BF).astype(F32)[:, 0, :]
    rmax = jnp.max(r)
    pos = lax.broadcasted_iota(I32, (NB, BQ), 0) * BQ + lax.broadcasted_iota(I32, (NB, BQ), 1)
    idx = jnp.min(jnp.where(r == rmax, pos, S))
    idx = jnp.minimum(idx, S - 1)
    base = pl.multiple_of((idx // 16) * 16, 16)
    slab = _layernorm_bf16(x_s[pl.ds(base, 16), :].astype(F32))
    rowsel = lax.broadcasted_iota(I32, (16, 1), 0) == (idx - base)
    xsel = jnp.where(rowsel, slab.astype(F32), 0.0)
    xsel = jnp.sum(xsel, axis=0, keepdims=True)
    xsel16 = jnp.broadcast_to(xsel, (16, D)).astype(BF)
    c_wg.wait()
    c_wu.wait()
    c_wd.wait()
    g = lax.dot_general(xsel16, wgt_s[...], NT, preferred_element_type=F32).astype(BF).astype(F32)
    u = lax.dot_general(xsel16, wut_s[...], NT, preferred_element_type=F32).astype(BF).astype(F32)
    g = (g * jax.nn.sigmoid(g)).astype(BF).astype(F32)
    hmid = (g * u).astype(BF)
    y = jnp.dot(hmid, wd_s[...], preferred_element_type=F32).astype(BF).astype(F32)
    rs = jax.nn.sigmoid(jnp.full((1, D), rmax, F32)).astype(BF).astype(F32)
    y = (y[0:1, :] * rs).astype(BF).astype(F32)
    rbase = pl.multiple_of((idx // 8) * 8, 8)
    rsel = lax.broadcasted_iota(I32, (8, 1), 0) == (idx - rbase)
    res_s[pl.ds(rbase, 8), :] = res_s[pl.ds(rbase, 8), :] + jnp.where(rsel, y, 0.0)

    row = lax.broadcasted_iota(I32, (64, 128), 0)
    col = lax.broadcasted_iota(I32, (64, 128), 1)
    maskd = row <= (col & 63)
    zeros16 = jnp.zeros((16, 128), I32)
    zhalf = jnp.zeros((64, 128), F32)
    lo = lax.broadcasted_iota(I32, (8, 128), 1) < 64

    def qk(b, u, nav, g8, par):
        kr0 = (2 * b + u - nav) * 32
        if not isinstance(b, int):
            kr0 = pl.multiple_of(kr0, 32)
        kall = k_s[g8, pl.ds(kr0, 32 * (nav + 1)), :]
        if nav == 4:
            pieces = []
            for i in range(4):
                pieces.append(kall[i * 8:(i + 1) * 8])
                pieces.append(kall[128 + i * 8:128 + (i + 1) * 8])
            pieces.append(kall[32:128])
            kall = jnp.concatenate(pieces, axis=0)
        cols = []
        for p in range(4):
            qh = q_s[b, u, 4 * g8 + p]
            cols.append(jnp.concatenate([zeros16] * p + [qh] + [zeros16] * (3 - p), axis=0))
        qm = _unpack(jnp.concatenate(cols, axis=1))
        st = jnp.dot(_unpack(kall), qm, preferred_element_type=F32)
        nmid = min(nav, 3)
        ms = []
        for p in range(4):
            sj = st[:, p * 128:(p + 1) * 128]
            if nav == 4:
                comb = jnp.concatenate([
                    jnp.where(maskd[i * 16:(i + 1) * 16], sj[i * 32 + 16:i * 32 + 32], sj[i * 32:i * 32 + 16])
                    for i in range(4)], axis=0)
                mid = sj[128:320]
            else:
                comb = jnp.where(maskd, sj[nav * 64:], -1e30)
                mid = sj[0:nav * 64]
            m = jnp.max(comb.reshape(8, 8, 128), axis=0)
            s_s[par, p, 0:64, :] = comb
            if nmid:
                s_s[par, p, 64:64 + 64 * nmid, :] = mid
                m = jnp.maximum(m, jnp.max(mid.reshape(8 * nmid, 8, 128), axis=0))
            ms.append(jnp.max(m, axis=0, keepdims=True))
        return ms

    def pv(b, u, nav, g8, par, ms):
        s = 2 * b + u
        nmid = min(nav, 3)
        xs = []
        for p in range(4):
            m = ms[p]
            pc = jnp.exp2(s_s[par, p, 0:64, :] - m)
            l = jnp.sum(pc.reshape(8, 8, 128), axis=0)
            halves = {}
            if nav == 4:
                halves[0] = jnp.where(maskd, pc, 0.0)
                halves[-4] = jnp.where(maskd, 0.0, pc)
            else:
                halves[0] = pc
            if nmid:
                pm = jnp.exp2(s_s[par, p, 64:64 + 64 * nmid, :] - m)
                l = l + jnp.sum(pm.reshape(8 * nmid, 8, 128), axis=0)
                for i in range(nmid):
                    halves[-nmid + i] = pm[i * 64:(i + 1) * 64]
            l = jnp.sum(l, axis=0, keepdims=True)
            ov = None
            P = 4 * g8 + p
            for db in range(-2, 1):
                o0, o1 = 2 * db - u, 2 * db + 1 - u
                if o0 not in halves and o1 not in halves:
                    continue
                pt = jnp.concatenate([halves.get(o0, zhalf), halves.get(o1, zhalf)], axis=0).astype(BF)
                vv = _unpack(v_s[b + db, P * 16:(P + 1) * 16, :])
                part = jnp.dot(vv, pt, preferred_element_type=F32)
                ov = part if ov is None else ov + part
            rc = pl.reciprocal(l, approx=True)
            rc = rc * (2.0 - l * rc)
            o = ov * rc
            xs.append((_pack(o[0:16]), _pack(o[16:32])))
        return xs

    def put_o(b, g8, xs0, xs1):
        for p in range(4):
            a = jnp.where(lo, xs0[p][0], xs1[p][1])
            bb = pltpu.roll(jnp.where(lo, xs1[p][0], xs0[p][1]), 64, axis=1)
            h0 = 8 * g8 + 2 * p
            ot_s[b % 2, h0 * 8:(h0 + 1) * 8, :] = jnp.where(lo, a, bb)
            ot_s[b % 2, (h0 + 1) * 8:(h0 + 2) * 8, :] = jnp.where(lo, bb, a)

    def out_proj(b):
        t0 = b * BQ if isinstance(b, int) else pl.multiple_of(b * BQ, BQ)
        a = lax.dot_general(_unpack(ot_s[b % 2]), _unpack(wo_s[...]), TN, preferred_element_type=F32)
        o_s[pl.ds(t0, BQ), :] = (res_s[pl.ds(t0, BQ), :] + a).astype(BF)

    def o_copy(b):
        t0 = b * BQ if isinstance(b, int) else pl.multiple_of(b * BQ, BQ)
        return pltpu.make_async_copy(o_s.at[pl.ds(t0, BQ), :], o_hbm.at[pl.ds(t0, BQ), :], sem_o)

    def nav_of(b, u):
        return min(2 * b + u, 4) if isinstance(b, int) else 4

    steps = [(g8, u) for g8 in range(4) for u in range(2)]

    def block(b, ms, has_next, prev_out):
        xs0 = None
        for i, (g8, u) in enumerate(steps):
            if i + 1 < 8:
                g8n, un = steps[i + 1]
                ms_next = qk(b, un, nav_of(b, un), g8n, (i + 1) % 2)
            elif has_next:
                ms_next = qk(b + 1, 0, nav_of(b + 1, 0), 0, 0)
            else:
                ms_next = None
            if i == OPG and prev_out:
                out_proj(b - 1)
            xs = pv(b, u, nav_of(b, u), g8, i % 2, ms)
            if u == 0:
                xs0 = xs
            else:
                put_o(b, g8, xs0, xs)
            ms = ms_next
        return ms

    ms = qk(0, 0, 0, 0, 0)
    ms = block(0, ms, True, False)
    ms = block(1, ms, True, True)
    o_copy(0).start()

    def p2(b, ms):
        ms = block(b, list(ms), True, True)
        o_copy(b - 1).start()
        return tuple(ms)
    ms = lax.fori_loop(2, NB - 1, p2, tuple(ms))
    block(NB - 1, list(ms), False, True)
    o_copy(NB - 2).start()
    out_proj(NB - 1)
    o_copy(NB - 1).start()
    pltpu.make_async_copy(o_s, o_hbm, sem_o).wait()


@jax.jit
def pallas_parallel_sum__sliding_block__moe_arch_mod__prompt_kernel(
    A_x, A_wqkv, A_wo, B_x, B_w_r, B_w_gate, B_w_up, B_w_down,
):
    del B_x
    hbm = pl.BlockSpec(memory_space=pltpu.HBM)
    out = pl.pallas_call(
        kernel,
        out_shape=jax.ShapeDtypeStruct((S, D), BF),
        in_specs=[hbm] * 7,
        out_specs=hbm,
        scratch_shapes=[
            pltpu.VMEM((S + BQ, D), BF),
            pltpu.VMEM((3, D, D), BF),
            pltpu.VMEM((D, D), BF),
            pltpu.VMEM((1, D), BF),
            pltpu.VMEM((F, D), BF),
            pltpu.VMEM((F, D), BF),
            pltpu.VMEM((F, D), BF),
            pltpu.VMEM((HB, D), I32),
            pltpu.VMEM((HB, D), I32),
            pltpu.VMEM((S + BQ, D), F32),
            pltpu.VMEM((4, S // 2, 128), I32),
            pltpu.VMEM((NB, D // 2, BQ), I32),
            pltpu.VMEM((NB, 2, 16, 16, 128), I32),
            pltpu.VMEM((D // 2, D), I32),
            pltpu.VMEM((520, D), I32),
            pltpu.VMEM((D // 2, D), I32),
            pltpu.VMEM((2, D // 2, BQ), I32),
            pltpu.VMEM((NB, 8, BQ), F32),
            pltpu.VMEM((2, 4, 256, 128), F32),
            pltpu.VMEM((S, D), BF),
            pltpu.SemaphoreType.DMA((NB + 1,)),
            pltpu.SemaphoreType.DMA((8,)),
            pltpu.SemaphoreType.DMA(()),
        ],
        compiler_params=pltpu.CompilerParams(vmem_limit_bytes=100 * 2**20),
    )(A_x.reshape(S, D), A_wqkv, A_wo, B_w_r.reshape(1, D), B_w_gate.T, B_w_up.T, B_w_down)
    return out.reshape(1, S, D)
```

```python
import functools, math
import numpy as np
import jax
import jax.numpy as jnp
from jax import lax
import jax.experimental.pallas as pl
import jax.experimental.pallas.tpu as pltpu

S, D, H, DH, W, F = 2048, 512, 32, 16, 256, 1376
BQ = 128
HB = BQ // 2
NB = S // BQ
BF = jnp.bfloat16
F32 = jnp.float32
I32 = jnp.int32
NT = (((1,), (1,)), ((), ()))
TN = (((0,), (0,)), ((), ()))
QSCALE = (DH ** -0.5) * math.log2(math.e)
U1 = 2
OPG = 0
FPOS = 1
OPG1 = 7
LAST = 1
OPGL = 7
DORD = 6
PV = 1
FA = (2, None)
FR = (0, 8)
U2 = 2
MODE = 5


def _pack(v):
    return pltpu.bitcast(v.astype(BF), I32)


def _unpack(v):
    return pltpu.bitcast(v, BF)


def _layernorm_bf16(xf):
    mean = jnp.mean(xf, axis=-1, keepdims=True)
    c = xf - mean
    var = jnp.mean(c * c, axis=-1, keepdims=True)
    m = mean.astype(BF).astype(F32)
    v = var.astype(BF).astype(F32)
    d = (xf - m).astype(BF).astype(F32)
    s = jnp.sqrt((v + 1e-5).astype(BF).astype(F32)).astype(BF).astype(F32)
    return (d / s).astype(BF)


def kernel(x_hbm, wqkv_hbm, wo_hbm, wr_hbm, wgt_hbm, wut_hbm, wd_hbm, o_hbm,
           x_s, wqkv_s, wo_in, wr_s, wgt_s, wut_s, wd_s,
           xa_s, xb_s, x0_s, x1_s, res_s, k_s, v_s, q_s, wk_s, wt_s, wo_s, ot_s, r_s, s_s, o_s, xr_s,
           sem_x, sem_w, sem_o):
    def x_copy(b):
        t0 = b * BQ if isinstance(b, int) else pl.multiple_of(b * BQ, BQ)
        src0 = min(b, NB - 1) * BQ if isinstance(b, int) else pl.multiple_of(jnp.minimum(b, NB - 1) * BQ, BQ)
        return pltpu.make_async_copy(x_hbm.at[pl.ds(src0, BQ), :], x_s.at[pl.ds(t0, BQ), :], sem_x.at[b])

    def w_copy(i):
        return pltpu.make_async_copy(wqkv_hbm.at[:, i * D:(i + 1) * D], wqkv_s.at[i], sem_w.at[i])

    c_wr = pltpu.make_async_copy(wr_hbm, wr_s, sem_w.at[3])
    c_wo = pltpu.make_async_copy(wo_hbm, wo_in, sem_w.at[4])
    c_wg = pltpu.make_async_copy(wgt_hbm, wgt_s, sem_w.at[5])
    c_wu = pltpu.make_async_copy(wut_hbm, wut_s, sem_w.at[6])
    c_wd = pltpu.make_async_copy(wd_hbm, wd_s, sem_w.at[7])

    early = {'r': c_wr, 'k': w_copy(1), 'q': w_copy(0), 'v': w_copy(2),
             '0': x_copy(0), '1': x_copy(1), '2': x_copy(2), '3': x_copy(3)}
    for c in ['01qrv2k3', '0q1rv2k3', '01qvr2k3', '01q2rvk3', '01qrvk23', '10qrv2k3', 'r01qv2k3'][DORD]:
        early[c].start()

    def ln_rows(b, dst, r0, n):
        t0 = b * BQ + r0 if isinstance(b, int) else pl.multiple_of(b * BQ + r0, 16)
        xf = x_s[pl.ds(t0, n), :].astype(F32)
        xn = _layernorm_bf16(xf)
        xp = pltpu.bitcast(xn, I32)
        dst[r0 // 2:(r0 + n) // 2, :] = xp
        res_s[pl.ds(t0, n), :] = xf + xn.astype(F32)
        z = xp[0:8, 0:128]
        for i in range(n // 16):
            for j in range(4):
                if i or j:
                    z = z | xp[i * 8:(i + 1) * 8, j * 128:(j + 1) * 128]
        return jnp.minimum(z & 0x7FFFFFFF, 0)

    lo8 = lax.broadcasted_iota(I32, (1, 8, 128), 2) < 64

    def k_proj(b, xn):
        h0 = b * HB if isinstance(b, int) else pl.multiple_of(b * HB, HB)
        kk = jnp.dot(xn, _unpack(wk_s[...]), preferred_element_type=F32)
        for g8 in range(4):
            k_s[g8, pl.ds(h0, HB), :] = _pack(kk[:, g8 * 128:(g8 + 1) * 128])

    def qv_proj(b, xn, c, z):
        r0, r1 = c * 128, (c + 1) * 128 + (8 if c == 3 else 0)
        if z is None:
            w = wt_s[r0:r1, :]
        else:
            first = wt_s[r0:r0 + 8, :]
            first = jnp.concatenate([first[:, 0:128] | z, first[:, 128:]], axis=1)
            w = jnp.concatenate([first, wt_s[r0 + 8:r1, :]], axis=0)
        o = lax.dot_general(_unpack(w), xn, NT, preferred_element_type=F32)
        if c < 2:
            qp = _pack(o * QSCALE).reshape(8, 2, 8, 128)
            qr = pltpu.roll(qp, 64, axis=3)
            q_s[b, 0, c * 8:(c + 1) * 8, 0:8, :] = jnp.where(lo8, qp[:, 0], 0)
            q_s[b, 0, c * 8:(c + 1) * 8, 8:16, :] = jnp.where(lo8, 0, qr[:, 1])
            q_s[b, 1, c * 8:(c + 1) * 8, 0:8, :] = jnp.where(lo8, qr[:, 0], 0)
            q_s[b, 1, c * 8:(c + 1) * 8, 8:16, :] = jnp.where(lo8, 0, qp[:, 1])
        else:
            v_s[b, (c - 2) * 128:(c - 1) * 128, :] = _pack(o[0:256])
            if c == 3:
                r_s[b] = o[256:264]

    def proj_block(b, src, dst):
        xn = _unpack(src[...])
        k_proj(b, xn)
        for c in range(4):
            qv_proj(b, xn, c, ln_rows(b + 1, dst, c * 32, 32))

    x_copy(0).wait()
    if PV == 1:
        x_copy(1).wait()
    ln_rows(0, x0_s, 0, BQ)
    if PV == 0:
        x_copy(1).wait()
    ln_rows(1, x1_s, 0, BQ)
    w_copy(0).wait()
    c_wr.wait()
    for b in range(4, NB + 1):
        x_copy(b).start()
    c_wo.start()
    c_wg.start()
    c_wu.start()
    c_wd.start()
    wt_s[0:256, :] = pltpu.bitcast(wqkv_s[0].T, I32)
    wt_s[512:520, :] = pltpu.bitcast(jnp.broadcast_to(wr_s[...].reshape(1, D), (16, D)), I32)
    for b, src in ((0, x0_s), (1, x1_s)):
        for c in range(2):
            qv_proj(b, _unpack(src[...]), c, None)
    w_copy(2).wait()
    x_copy(2).wait()
    wt_s[256:512, :] = pltpu.bitcast(wqkv_s[2].T, I32)
    for b, src in ((0, x0_s), (1, x1_s)):
        for c in range(2, 4):
            qv_proj(b, _unpack(src[...]), c, ln_rows(2, xa_s, (2 * b + c - 2) * 32, 32))
    w_copy(1).wait()
    wk_s[...] = pltpu.bitcast(wqkv_s[1], I32)
    k_proj(0, _unpack(x0_s[...]))
    k_proj(1, _unpack(x1_s[...]))

    def p1(i, c):
        for j in range(U1):
            x_copy(2 + U1 * i + j + 1).wait()
        for j in range(U1):
            proj_block(2 + U1 * i + j, (xa_s, xb_s)[j % 2], (xa_s, xb_s)[(j + 1) % 2])
        return c
    lax.fori_loop(0, (NB - 2) // U1, p1, 0)

    c_wo.wait()
    c_wg.wait()
    c_wu.wait()
    c_wd.wait()
    wo_s[...] = pltpu.bitcast(wo_in[...], I32)

    r = r_s[...].astype(BF).astype(F32)[:, 0, :]
    rmax = jnp.max(r)
    pos = lax.broadcasted_iota(I32, (NB, BQ), 0) * BQ + lax.broadcasted_iota(I32, (NB, BQ), 1)
    idx = jnp.min(jnp.where(r == rmax, pos, S))
    idx = jnp.minimum(idx, S - 1)
    bstar = idx // BQ
    base = pl.multiple_of((idx // 16) * 16, 16)
    rowsel = lax.broadcasted_iota(I32, (16, 1), 0) == (idx - base)
    slab = _layernorm_bf16(x_s[pl.ds(base, 16), :].astype(F32))
    xr_s[...] = jnp.broadcast_to(jnp.sum(jnp.where(rowsel, slab.astype(F32), 0.0), axis=0, keepdims=True), (8, D))

    def rnd(v):
        return v.astype(BF).astype(F32)

    yacc = [None]
    FP = 32
    NFP = F // FP

    def ffn_piece(k, rel=None):
        f0 = k * FP if isinstance(k, int) else pl.multiple_of(k * FP, FP)
        xr = xr_s[...]
        if rel is not None:
            xr = pltpu.bitcast(pltpu.bitcast(xr, I32) | jnp.concatenate([rel] * 4, axis=1), F32)
        xr = xr[0:1, :]
        g = rnd(jnp.sum(wgt_s[pl.ds(f0, FP), :].astype(F32) * xr, axis=1, keepdims=True))
        u = rnd(jnp.sum(wut_s[pl.ds(f0, FP), :].astype(F32) * xr, axis=1, keepdims=True))
        h = rnd(rnd(g * jax.nn.sigmoid(g)) * u)
        yp = wd_s[pl.ds(f0, FP), :].astype(F32) * h
        yp = jnp.sum(yp.reshape(FP // 8, 8, D), axis=0)
        yacc[0] = yacc[0] + yp
        return pltpu.bitcast(yp[:, 0:128], I32)

    def ffn_group(k0, n, zero, rel=None):
        w = None
        for p in range(n):
            v = ffn_piece(k0 + p, rel)
            w = v if w is None else w | v
        return w & zero

    row = lax.broadcasted_iota(I32, (64, 128), 0)
    col = lax.broadcasted_iota(I32, (64, 128), 1)
    maskd = row <= (col & 63)
    zeros16 = jnp.zeros((16, 128), I32)
    zhalf = jnp.zeros((64, 128), F32)
    lo = lax.broadcasted_iota(I32, (8, 128), 1) < 64

    def qk(b, u, nav, g8, par, z=None):
        kr0 = (2 * b + u - nav) * 32
        if not isinstance(b, int):
            kr0 = pl.multiple_of(kr0, 32)
        kall = k_s[g8, pl.ds(kr0, 32 * (nav + 1)), :]
        if z is not None:
            kall = jnp.concatenate([kall[0:8] | z, kall[8:]], axis=0)
        if nav == 4:
            pieces = []
            for i in range(4):
                pieces.append(kall[i * 8:(i + 1) * 8])
                pieces.append(kall[128 + i * 8:128 + (i + 1) * 8])
            pieces.append(kall[32:128])
            kall = jnp.concatenate(pieces, axis=0)
        cols = []
        for p in range(4):
            qh = q_s[b, u, 4 * g8 + p]
            cols.append(jnp.concatenate([zeros16] * p + [qh] + [zeros16] * (3 - p), axis=0))
        qm = _unpack(jnp.concatenate(cols, axis=1))
        st = jnp.dot(_unpack(kall), qm, preferred_element_type=F32)
        nmid = min(nav, 3)
        ms = []
        for p in range(4):
            sj = st[:, p * 128:(p + 1) * 128]
            if nav == 4:
                comb = jnp.concatenate([
                    jnp.where(maskd[i * 16:(i + 1) * 16], sj[i * 32 + 16:i * 32 + 32], sj[i * 32:i * 32 + 16])
                    for i in range(4)], axis=0)
                mid = sj[128:320]
            else:
                comb = jnp.where(maskd, sj[nav * 64:], -1e30)
                mid = sj[0:nav * 64]
            m = jnp.max(comb.reshape(8, 8, 128), axis=0)
            s_s[par, p, 0:64, :] = comb
            if nmid:
                s_s[par, p, 64:64 + 64 * nmid, :] = mid
                m = jnp.maximum(m, jnp.max(mid.reshape(8 * nmid, 8, 128), axis=0))
            ms.append(jnp.max(m, axis=0, keepdims=True))
        return ms

    def pv(b, u, nav, g8, par, ms):
        s = 2 * b + u
        nmid = min(nav, 3)
        xs = []
        for p in range(4):
            m = ms[p]
            pc = jnp.exp2(s_s[par, p, 0:64, :] - m)
            l = jnp.sum(pc.reshape(8, 8, 128), axis=0)
            halves = {}
            if nav == 4:
                halves[0] = jnp.where(maskd, pc, 0.0)
                halves[-4] = jnp.where(maskd, 0.0, pc)
            else:
                halves[0] = pc
            if nmid:
                pm = jnp.exp2(s_s[par, p, 64:64 + 64 * nmid, :] - m)
                l = l + jnp.sum(pm.reshape(8 * nmid, 8, 128), axis=0)
                for i in range(nmid):
                    halves[-nmid + i] = pm[i * 64:(i + 1) * 64]
            l = jnp.sum(l, axis=0, keepdims=True)
            ov = None
            P = 4 * g8 + p
            for db in range(-2, 1):
                o0, o1 = 2 * db - u, 2 * db + 1 - u
                if o0 not in halves and o1 not in halves:
                    continue
                pt = jnp.concatenate([halves.get(o0, zhalf), halves.get(o1, zhalf)], axis=0).astype(BF)
                vv = _unpack(v_s[b + db, P * 16:(P + 1) * 16, :])
                part = jnp.dot(vv, pt, preferred_element_type=F32)
                ov = part if ov is None else ov + part
            rc = pl.reciprocal(l, approx=True)
            rc = rc * (2.0 - l * rc)
            o = ov * rc
            xs.append((_pack(o[0:16]), _pack(o[16:32])))
        return xs

    def put_o(b, g8, xs0, xs1):
        for p in range(4):
            a = jnp.where(lo, xs0[p][0], xs1[p][1])
            bb = pltpu.roll(jnp.where(lo, xs1[p][0], xs0[p][1]), 64, axis=1)
            h0 = 8 * g8 + 2 * p
            ot_s[b % 2, h0 * 8:(h0 + 1) * 8, :] = jnp.where(lo, a, bb)
            ot_s[b % 2, (h0 + 1) * 8:(h0 + 2) * 8, :] = jnp.where(lo, bb, a)

    def out_proj(b):
        t0 = b * BQ if isinstance(b, int) else pl.multiple_of(b * BQ, BQ)
        a = lax.dot_general(_unpack(ot_s[b % 2]), _unpack(wo_s[...]), TN, preferred_element_type=F32)
        o32 = res_s[pl.ds(t0, BQ), :] + a
        res_s[pl.ds(t0, BQ), :] = o32
        o_s[pl.ds(t0, BQ), :] = o32.astype(BF)
        return pltpu.bitcast(a[0:8, 0:128], I32)

    def o_copy(b):
        t0 = b * BQ if isinstance(b, int) else pl.multiple_of(b * BQ, BQ)
        return pltpu.make_async_copy(o_s.at[pl.ds(t0, BQ), :], o_hbm.at[pl.ds(t0, BQ), :], sem_o)

    def nav_of(b, u):
        return min(2 * b + u, 4) if isinstance(b, int) else 4

    steps = [(g8, u) for g8 in range(4) for u in range(2)]

    def block(b, ms, nb, prev_out, last=False, fk=None):
        xs0 = None
        relv = [None]
        if fk is not None:
            zero = jnp.minimum(fk[0], 0)
        for i, (g8, u) in enumerate(steps):
            def next_qk():
                if i + 1 < 8:
                    g8n, un = steps[i + 1]
                    z = None
                    if fk is not None and i == FA[fk[1]]:
                        z = ffn_group(fk[0], 3, zero, relv[0])
                    return qk(b, un, nav_of(b, un), g8n, (i + 1) % 2, z)
                elif nb is not None:
                    return qk(nb, 0, nav_of(nb, 0), 0, 0)
                return None
            late = last and i == 7
            if not late:
                ms_next = next_qk()
            if i == prev_out:
                a0 = out_proj(b - 1)
                if fk is not None and FR[fk[1]] == 8:
                    ffn_group(fk[0], 3, zero, a0 & zero)
            xs = pv(b, u, nav_of(b, u), g8, i % 2, ms)
            if fk is not None and i == FR[fk[1]]:
                relv[0] = xs[3][1] & zero
            if fk is not None and FA[fk[1]] is None and i == FR[fk[1]]:
                ffn_group(fk[0], 3, zero, relv[0])
            if u == 0:
                xs0 = xs
            else:
                put_o(b, g8, xs0, xs)
            if late:
                ms_next = next_qk()
            ms = ms_next
        return ms

    def o_start(b):
        @pl.when(b != bstar)
        def _():
            o_copy(b).start()

    ms = qk(0, 0, 0, 0, 0)
    ms = block(0, ms, 1, None)
    yacc[0] = jnp.zeros((8, D), F32)
    ffn_piece(0)
    y0 = yacc[0]
    ms = block(1, ms, 2, OPG1)
    o_start(0)

    def p2(i, carry):
        ms = list(carry[:4])
        yacc[0] = carry[4]
        for j in range(U2):
            b = 2 + U2 * i + j
            ms = block(b, ms, jnp.minimum(b + 1, NB - 1), OPG if j < U2 - 1 else OPGL, LAST and j == U2 - 1,
                       fk=(1 + 3 * (U2 * i + j), j))
        for j in range(U2):
            o_start(2 + U2 * i + j - 1)
        return tuple(ms) + (yacc[0],)
    carry = lax.fori_loop(0, (NB - 2) // U2, p2, tuple(ms) + (y0,))
    out_proj(NB - 1)

    y = rnd(jnp.sum(carry[4], axis=0, keepdims=True))
    rs = rnd(jax.nn.sigmoid(jnp.full((1, D), rmax, F32)))
    y = rnd(y * rs)
    o_s[pl.ds(base, 16), :] = (res_s[pl.ds(base, 16), :] + jnp.where(rowsel, y, 0.0)).astype(BF)
    o_copy(NB - 1).start()

    @pl.when(bstar != NB - 1)
    def _():
        o_copy(bstar).start()
    pltpu.make_async_copy(o_s, o_hbm, sem_o).wait()


@jax.jit
def pallas_parallel_sum__sliding_block__moe_arch_mod__prompt_kernel(
    A_x, A_wqkv, A_wo, B_x, B_w_r, B_w_gate, B_w_up, B_w_down,
):
    del B_x
    hbm = pl.BlockSpec(memory_space=pltpu.HBM)
    out = pl.pallas_call(
        kernel,
        out_shape=jax.ShapeDtypeStruct((S, D), BF),
        in_specs=[hbm] * 7,
        out_specs=hbm,
        scratch_shapes=[
            pltpu.VMEM((S + BQ, D), BF),
            pltpu.VMEM((3, D, D), BF),
            pltpu.VMEM((D, D), BF),
            pltpu.VMEM((D,), BF),
            pltpu.VMEM((F, D), BF),
            pltpu.VMEM((F, D), BF),
            pltpu.VMEM((F, D), BF),
            pltpu.VMEM((HB, D), I32),
            pltpu.VMEM((HB, D), I32),
            pltpu.VMEM((HB, D), I32),
            pltpu.VMEM((HB, D), I32),
            pltpu.VMEM((S + BQ, D), F32),
            pltpu.VMEM((4, S // 2, 128), I32),
            pltpu.VMEM((NB, D // 2, BQ), I32),
            pltpu.VMEM((NB, 2, 16, 16, 128), I32),
            pltpu.VMEM((D // 2, D), I32),
            pltpu.VMEM((520, D), I32),
            pltpu.VMEM((D // 2, D), I32),
            pltpu.VMEM((2, D // 2, BQ), I32),
            pltpu.VMEM((NB, 8, BQ), F32),
            pltpu.VMEM((2, 4, 256, 128), F32),
            pltpu.VMEM((S, D), BF),
            pltpu.VMEM((8, D), F32),
            pltpu.SemaphoreType.DMA((NB + 1,)),
            pltpu.SemaphoreType.DMA((8,)),
            pltpu.SemaphoreType.DMA(()),
        ],
        compiler_params=pltpu.CompilerParams(vmem_limit_bytes=100 * 2**20),
    )(A_x.reshape(S, D), A_wqkv, A_wo, B_w_r, B_w_gate.T, B_w_up.T, B_w_down)
    return out.reshape(1, S, D)
```

```python
import functools, math
import numpy as np
import jax
import jax.numpy as jnp
from jax import lax
import jax.experimental.pallas as pl
import jax.experimental.pallas.tpu as pltpu

S, D, H, DH, W, F = 2048, 512, 32, 16, 256, 1376
BQ = 128
HB = BQ // 2
NB = S // BQ
BF = jnp.bfloat16
F32 = jnp.float32
I32 = jnp.int32
NT = (((1,), (1,)), ((), ()))
TN = (((0,), (0,)), ((), ()))
QSCALE = (DH ** -0.5) * math.log2(math.e)
NEG = -1e30
FP = 32
OPG = 2
OPGL = 6
FA0 = 4
FR0 = 2
FR1 = 8
LA = 2
NBUF = 2 * LA
ANCH = [(), (7, 15, 23), (3, 7, 11, 15, 19, 23), tuple(range(24)), (23,)][0]
LNS = [(1, 2, 3, 4), (0, 1, 2, 3), (2, 3, 4, 5), (0, 2, 4, 5)][0]
KSS = [[[0, 1, 2, 3], [4, 5, 6, 7], [8, 9, 10, 11], [12, 13, 14, 15]], [[0, 1, 2, 3, 4, 5, 6, 7], [], [8, 9, 10, 11, 12, 13, 14, 15], []]][1]
MIDS = [[[n] for n in range(16)], [[2 * n, 2 * n + 1] for n in range(8)] + [[]] * 8][0]
KS2 = [[[8 + g] for g in range(8)], [[], [], [], [8], [9, 10], [11, 12], [13, 14], [15]], [[], [], [], [8, 9], [10, 11], [12, 13], [14, 15], []], [[15], [], [], [8], [9], [10, 11], [12, 13], [14]], [[8, 9], [], [10, 11], [], [12, 13], [], [14, 15], []], [[], [], [], [8, 9], [10, 11], [12, 13], [14, 15], []]][2]
PRO1 = 0
KREL = 0
assert FA0 + LA < 8
OPGT = 6
SPLIT = 1
NOF = 0


def _pack(v):
    return pltpu.bitcast(v.astype(BF), I32)


def _pack_pi(v):
    n = v.shape[0] // 16
    v4 = v.reshape(n, 2, 8, v.shape[1])
    return pltpu.pack_elementwise([v4[:, 0], v4[:, 1]], packed_dtype=BF).reshape(8 * n, v.shape[1])


def _unpack(v):
    return pltpu.bitcast(v, BF)


def _rnd(v):
    return v.astype(BF).astype(F32)


def _layernorm(xf):
    mean = jnp.mean(xf, axis=-1, keepdims=True)
    c = xf - mean
    var = jnp.mean(c * c, axis=-1, keepdims=True)
    d = _rnd(xf - _rnd(mean))
    s = _rnd(jnp.sqrt(_rnd(_rnd(var) + 1e-5)))
    return d / s


def kernel(x_hbm, wqkv_hbm, wo_hbm, wr_hbm, wgt_hbm, wut_hbm, wd_hbm, o_hbm,
           x_s, wqkv_s, wo_in, wr_s, wgt_s, wut_s, wd_s,
           xn_s, res_s, ta_s, tb_s, ks_s, v_s, q_s, wt_s, wo_s, ot_s, r_s, s_s, o_s, xr_s,
           sem_x, sem_w, sem_o):
    def x_copy(b):
        t0 = b * BQ if isinstance(b, int) else pl.multiple_of(b * BQ, BQ)
        src0 = min(b, NB - 1) * BQ if isinstance(b, int) else pl.multiple_of(jnp.minimum(b, NB - 1) * BQ, BQ)
        return pltpu.make_async_copy(x_hbm.at[pl.ds(src0, BQ), :], x_s.at[pl.ds(t0, BQ), :], sem_x.at[b])

    def w_copy(i):
        return pltpu.make_async_copy(wqkv_hbm.at[:, i * D:(i + 1) * D], wqkv_s.at[i], sem_w.at[i])

    c_wr = pltpu.make_async_copy(wr_hbm, wr_s, sem_w.at[3])
    c_wo = pltpu.make_async_copy(wo_hbm, wo_in, sem_w.at[4])
    c_wg = pltpu.make_async_copy(wgt_hbm, wgt_s, sem_w.at[5])
    c_wu = pltpu.make_async_copy(wut_hbm, wut_s, sem_w.at[6])
    c_wd = pltpu.make_async_copy(wd_hbm, wd_s, sem_w.at[7])

    for c in (c_wr, x_copy(0), x_copy(1), w_copy(1), w_copy(0), x_copy(2), w_copy(2), x_copy(3)):
        c.start()

    lane8 = lax.broadcasted_iota(I32, (8, 128), 1)
    zero8 = jnp.zeros((8, 128), I32)

    def ln_rows(b, slot, r0, n):
        t0 = b * BQ + r0 if isinstance(b, int) else pl.multiple_of(b * BQ + r0, 16)
        xf = x_s[pl.ds(t0, n), :].astype(F32)
        xn = _rnd(_layernorm(xf))
        xn_s[slot, 0, r0 // 2:(r0 + n) // 2, :] = _pack(xn)
        xn_s[slot, 1, r0 // 2:(r0 + n) // 2, :] = _pack_pi(xn)
        res_s[pl.ds(t0, n), :] = xf + xn
        return pltpu.bitcast(xn[n - 8:n, 384:512], I32)

    def proj(b, slot, kind, c, z=None):
        r0 = kind * 256 + c * 128
        r1 = r0 + 128 + (8 if (kind == 2 and c == 1) else 0)
        xn = _unpack(xn_s[slot, 1 if kind == 2 else 0])
        w = wt_s[r0:r1, :]
        if z is not None:
            w = jnp.concatenate([jnp.concatenate([w[0:8, 0:128] | z, w[0:8, 128:]], axis=1), w[8:]], axis=0)
        o = lax.dot_general(_unpack(w), xn, NT, preferred_element_type=F32)
        if kind == 0:
            q_s[b, c * 128:(c + 1) * 128, :] = _pack_pi(o * QSCALE)
        elif kind == 1:
            return _pack_pi(o)
        else:
            v_s[b, c * 128:(c + 1) * 128, :] = _pack(o[0:256])
            if c == 1:
                r_s[b] = o[256:264]

    jbit = [((lane8 >> 4) & (1 << k)) != 0 for k in range(3)]

    def build_ks(b, pairs, slabs, t_prev, t_cur):
        row0 = b * HB if isinstance(b, int) else pl.multiple_of(b * HB, HB)
        for p in pairs:
            hs = (2 * p, 2 * p + 1)
            if slabs is not None:
                rows = [slabs[h // 16][(h % 16) * 8:(h % 16 + 1) * 8] for h in hs for _ in range(8)]
                tt = pltpu.bitcast(_unpack(jnp.concatenate(rows, axis=0)).T, I32)
            for n, h in enumerate(hs):
                if slabs is not None:
                    cur = tt[:, n * 128:(n + 1) * 128]
                    t_cur[h] = cur
                prev = None if t_prev is None else t_prev[h]
                g = [None if prev is None else prev[8 * i:8 * i + 8] for i in range(8)] + \
                    [None if slabs is None else cur[8 * i:8 * i + 8] for i in range(7)]
                for k in (2, 1, 0):
                    sh = 1 << k
                    nxt = []
                    for i in range(len(g) - sh):
                        lo, hi = g[i], g[i + sh]
                        if lo is None and hi is None:
                            nxt.append(None)
                        else:
                            nxt.append(jnp.where(jbit[k], zero8 if hi is None else hi, zero8 if lo is None else lo))
                    g = nxt
                ks_s[h, pl.ds(row0, HB), :] = jnp.concatenate([zero8 if x is None else x for x in g], axis=0)

    def t_weight(i, kind):
        wt_s[kind * 256:(kind + 1) * 256, :] = pltpu.bitcast(wqkv_s[i].T, I32)

    x_copy(0).wait()
    x_copy(1).wait()
    ln_rows(0, 2, 0, BQ)
    ln_rows(1, 3, 0, BQ)
    w_copy(1).wait()
    c_wr.wait()
    for b in range(4, NB + 1):
        x_copy(b).start()
    c_wo.start()
    c_wg.start()
    c_wu.start()
    c_wd.start()
    t_weight(1, 1)
    wt_s[768:776, :] = pltpu.bitcast(jnp.broadcast_to(wr_s[...].reshape(1, D), (16, D)), I32)
    kt = [[proj(b, 2 + b, 1, c) for c in range(2)] for b in (0, 1)]
    w_copy(0).wait()
    x_copy(2).wait()
    t_weight(0, 0)
    xb = pltpu.bitcast(x_s[0:16, 0:128], I32)
    zvec = (xb * xb + xb) & 1
    def pro_builds(n):
        build_ks(0, range(2 * n, 2 * n + 2), kt[0], None, ta_s)
        build_ks(1, range(2 * n, 2 * n + 2), kt[1], ta_s, tb_s)

    lnz = [None, ln_rows(2, 0, 0, 64), ln_rows(2, 0, 64, 32), ln_rows(2, 0, 96, 32)]
    for b in (0, 1):
        for c in range(2):
            n = 2 * b + c
            pro_builds(n)
            proj(b, 2 + b, 0, c, None if lnz[n] is None else lnz[n] & zvec)
    w_copy(2).wait()
    t_weight(2, 2)
    for b in (0, 1):
        for c in range(2):
            pro_builds(4 + 2 * b + c)
            proj(b, 2 + b, 2, c)

    def proj_block(b, src, dst, t_prev, t_cur):
        cur = []
        n = 0
        for kind in (1, 0, 2):
            for c in range(2):
                if n in LNS:
                    ln_rows(b + 1, dst, LNS.index(n) * 32, 32)
                if n >= 2:
                    build_ks(b, KSS[n - 2], cur, t_prev, t_cur)
                o = proj(b, src, kind, c)
                if kind == 1:
                    cur.append(o)
                n += 1

    def p1(i, c):
        for j in range(2):
            x_copy(2 + 2 * i + j + 1).wait()
        for j in range(2):
            proj_block(2 + 2 * i + j, j, 1 - j, (tb_s, ta_s)[j], (ta_s, tb_s)[j])
        return c
    lax.fori_loop(0, (NB - 2) // 2, p1, 0)

    c_wo.wait()
    c_wg.wait()
    c_wu.wait()
    c_wd.wait()
    wo_s[...] = _pack_pi(wo_in[...].astype(F32))
    r = _rnd(r_s[...])[:, 0, :]
    rmax = jnp.max(r)
    ln = lax.broadcasted_iota(I32, (NB, BQ), 1)
    pos = lax.broadcasted_iota(I32, (NB, BQ), 0) * BQ + (ln & -16) + ((ln & 15) >> 1) + 8 * (ln & 1)
    idx = jnp.min(jnp.where(r == rmax, pos, S))
    idx = jnp.minimum(idx, S - 1)
    bstar = idx // BQ
    base = pl.multiple_of((idx // 16) * 16, 16)
    rowsel = lax.broadcasted_iota(I32, (16, 1), 0) == (idx - base)
    slab = _rnd(_layernorm(x_s[pl.ds(base, 16), :].astype(F32)))
    xr_s[...] = jnp.broadcast_to(jnp.sum(jnp.where(rowsel, slab, 0.0), axis=0, keepdims=True), (8, D))

    yacc = [None]

    def ffn_piece(k, rel=None):
        f0 = k * FP if isinstance(k, int) else pl.multiple_of(k * FP, FP)
        xr = xr_s[...]
        if rel is not None:
            xr = pltpu.bitcast(pltpu.bitcast(xr, I32) | jnp.concatenate([rel] * 4, axis=1), F32)
        xr = xr[0:1, :]
        g = _rnd(jnp.sum(wgt_s[pl.ds(f0, FP), :].astype(F32) * xr, axis=1, keepdims=True))
        u = _rnd(jnp.sum(wut_s[pl.ds(f0, FP), :].astype(F32) * xr, axis=1, keepdims=True))
        h = _rnd(_rnd(g * jax.nn.sigmoid(g)) * u)
        yp = wd_s[pl.ds(f0, FP), :].astype(F32) * h
        yp = jnp.sum(yp.reshape(FP // 8, 8, D), axis=0)
        yacc[0] = yacc[0] + yp
        return pltpu.bitcast(yp[:, 0:128], I32)

    def ffn_group(k0, n, zero, rel=None):
        w = None
        for p in range(n):
            v = ffn_piece(k0 + p, rel)
            w = v if w is None else w | v
        return w & zero

    maskd = lax.broadcasted_iota(I32, (16, 128), 0) <= (lax.broadcasted_iota(I32, (16, 128), 1) & 15)
    lane16 = lax.broadcasted_iota(I32, (16, 128), 1)
    ones8 = jnp.full((8, 128), 0x3F803F80, I32)
    jmask = [(lane8 >> 4) == j for j in range(8)]

    dzero = jnp.minimum(idx, 0)

    def first_group(t):
        return max(9 - 8 * t, 0) if isinstance(t, int) else 0

    def qk(t, G, par, z=None):
        i0 = first_group(t)
        ms = []
        for jh in range(4):
            h = 4 * G + jh
            row0 = (t - 1) * HB + 8 * i0
            if not isinstance(t, int):
                row0 = pl.multiple_of(row0, HB)
            kall = ks_s[h, pl.ds(row0, 8 * (17 - i0)), :]
            if i0 == 0:
                kall = jnp.concatenate([kall[0:8], kall[128:136], kall[8:128]], axis=0)
            if z is not None and jh == 0:
                kall = jnp.concatenate([kall[0:8] | z, kall[8:]], axis=0)
            qh = q_s[t, h * 8:(h + 1) * 8, :]
            qm = jnp.concatenate([jnp.where(jmask[j], qh, 0) for j in range(8)], axis=0)
            st = jnp.dot(_unpack(kall), _unpack(qm), preferred_element_type=F32)
            if i0 == 0:
                comb = jnp.where(maskd, st[16:32], st[0:16])
                mid = st[32:272]
            else:
                nm = 16 - i0
                comb = jnp.where(maskd, st[16 * nm:], NEG)
                mid = jnp.concatenate([
                    jnp.where(lane16 >= 16 * (16 - 8 * t - i), st[16 * (i - i0):16 * (i - i0 + 1)], NEG)
                    for i in range(i0, 16)], axis=0)
            nm = mid.shape[0]
            m = jnp.maximum(jnp.max(comb.reshape(2, 8, 128), axis=0), jnp.max(mid.reshape(nm // 8, 8, 128), axis=0))
            s_s[par, jh, 0:16, :] = comb
            s_s[par, jh, 16:16 + nm, :] = mid
            ms.append(jnp.max(m, axis=0, keepdims=True))
        return ms

    def unskew(plist):
        cur = plist
        for k in range(3):
            sh = 1 << k
            nxt = []
            for i in range(len(cur) + sh):
                a = cur[i - sh] if 0 <= i - sh < len(cur) else None
                b = cur[i] if i < len(cur) else None
                if a is None and b is None:
                    nxt.append(None)
                else:
                    nxt.append(jnp.where(jbit[k], zero8 if a is None else a, zero8 if b is None else b))
            cur = nxt
        return cur

    def softmax(t, G, par, ms):
        i0 = first_group(t)
        nm = 16 * (16 - max(i0, 1))
        us = []
        for jh in range(4):
            m = ms[jh]
            pc = jnp.exp2(s_s[par, jh, 0:16, :] - m)
            pm = _pack_pi(jnp.exp2(s_s[par, jh, 16:16 + nm, :] - m))
            plist = [None] * 17
            first_mid = 16 - nm // 16
            for i in range(nm // 16):
                plist[first_mid + i] = pm[8 * i:8 * i + 8]
            if i0 == 0:
                plist[0] = _pack_pi(jnp.where(maskd, 0.0, pc))
                plist[16] = _pack_pi(jnp.where(maskd, pc, 0.0))
            else:
                plist[16] = _pack_pi(pc)
            us.append(unskew(plist))
        return us

    def pv(t, G, us):
        os_ = []
        for jh in range(4):
            h = 4 * G + jh
            u = us[jh]
            ov = None
            for T in range(3):
                if isinstance(t, int) and t - 2 + T < 0:
                    continue
                tile = jnp.concatenate([zero8 if x is None else x for x in u[8 * T:8 * T + 8]], axis=0)
                vh = v_s[t - 2 + T, h * 8:(h + 1) * 8, :]
                vv = _unpack(jnp.concatenate([vh, ones8], axis=0))
                part = jnp.dot(vv, _unpack(tile), preferred_element_type=F32)
                ov = part if ov is None else ov + part
            l = ov[16:24]
            rc = pl.reciprocal(l, approx=True)
            rc = rc * (2.0 - l * rc)
            o = _pack_pi((ov[0:16].reshape(2, 8, 128) * rc).reshape(16, 128))
            ot_s[t % 2, h * 8:(h + 1) * 8, :] = o
            os_.append(o)
        return os_

    def anchor(us):
        z = None
        for u in us:
            for I in ANCH:
                if u[I] is not None:
                    z = u[I] if z is None else z | u[I]
        return z & dzero

    def out_proj(b):
        t0 = b * BQ if isinstance(b, int) else pl.multiple_of(b * BQ, BQ)
        a = lax.dot_general(_unpack(ot_s[b % 2]), _unpack(wo_s[...]), TN, preferred_element_type=F32)
        o32 = res_s[pl.ds(t0, BQ), :] + a
        res_s[pl.ds(t0, BQ), :] = o32
        o_s[pl.ds(t0, BQ), :] = o32.astype(BF)
        return pltpu.bitcast(a[0:8, 0:128], I32)

    def out_proj_part(b, g, last=False):
        a = lax.dot_general(_unpack(ot_s[b % 2, g * 64:(g + 1) * 64, :]), _unpack(wo_s[g * 64:(g + 1) * 64, :]),
                            TN, preferred_element_type=F32)
        o32 = res_s[b * BQ:(b + 1) * BQ, :] + a
        res_s[b * BQ:(b + 1) * BQ, :] = o32
        if last:
            o_s[b * BQ:(b + 1) * BQ, :] = o32.astype(BF)

    def o_copy(b):
        t0 = b * BQ if isinstance(b, int) else pl.multiple_of(b * BQ, BQ)
        return pltpu.make_async_copy(o_s.at[pl.ds(t0, BQ), :], o_hbm.at[pl.ds(t0, BQ), :], sem_o)

    def o_start(b):
        @pl.when(b != bstar)
        def _():
            o_copy(b).start()

    def block(t, pend, nt, prev_out, last=False, fk=None):
        rel = None
        krel = None
        pend = list(pend)
        if fk is not None:
            zero = dzero
        for G in range(8):
            def next_qk():
                n = G + LA
                if n < 8:
                    z = None
                    if fk is not None and fk[1] == 0 and G == FA0:
                        z = ffn_group(fk[0], 3, zero, rel)
                    if zs is not None:
                        z = zs if z is None else z | zs
                    return qk(t, n, n % NBUF, z)
                return None if nt is None else qk(nt, n - 8, n % NBUF, zs)
            late = last and G == 7
            if isinstance(t, int) and t < 2:
                build_ks(NB, MIDS[8 * t + G], None, tb_s, None)
            us = softmax(t, G, G % NBUF, pend.pop(0))
            zs = anchor(us) if ANCH else None
            if not late:
                pend.append(next_qk())
            if G == prev_out:
                a0 = out_proj(t - 1)
                if fk is not None and fk[1] == 1:
                    ffn_group(fk[0], 3, zero, a0 & zero)
            os_ = pv(t, G, us)
            if KREL:
                krel = os_[KREL - 1] & dzero
            if fk is not None and fk[1] == 0 and G == FR0:
                rel = os_[3] & zero
            if late:
                pend.append(next_qk())
            if isinstance(t, int) and t == NB - 1 and SPLIT and G in (3, 5, 7):
                out_proj_part(t, (G - 3) // 2)
        return pend

    pend = [qk(0, n, n % NBUF) for n in range(LA)]
    pend = block(0, pend, 1, None)
    yacc[0] = jnp.zeros((8, D), F32)
    ffn_piece(0)
    y0 = yacc[0]
    pend = block(1, pend, 2, 7, True)
    o_start(0)

    def p2(i, carry):
        pend = [list(carry[4 * n:4 * n + 4]) for n in range(LA)]
        yacc[0] = carry[-1]
        for j in range(2):
            t = 2 + 2 * i + j
            pend = block(t, pend, jnp.minimum(t + 1, NB - 1), OPG if j == 0 else OPGL, j == 1,
                         fk=None if NOF else (1 + 3 * (2 * i + j), j))
        for j in range(2):
            o_start(2 + 2 * i + j - 1)
        return tuple(m for ms in pend for m in ms) + (yacc[0],)
    carry = lax.fori_loop(0, (NB - 4) // 2, p2, tuple(m for ms in pend for m in ms) + (y0,))
    pend = [list(carry[4 * n:4 * n + 4]) for n in range(LA)]
    yacc[0] = carry[-1]
    pend = block(NB - 2, pend, NB - 1, OPG, fk=(37, 0))
    block(NB - 1, pend, None, OPGT, fk=(40, 1))
    o_start(NB - 3)
    o_start(NB - 2)
    ylast = yacc[0]
    if SPLIT:
        out_proj_part(NB - 1, 3, True)
    else:
        out_proj(NB - 1)

    y = _rnd(jnp.sum(ylast, axis=0, keepdims=True))
    rs = _rnd(jax.nn.sigmoid(jnp.full((1, D), rmax, F32)))
    y = _rnd(y * rs)
    o_s[pl.ds(base, 16), :] = (res_s[pl.ds(base, 16), :] + jnp.where(rowsel, y, 0.0)).astype(BF)
    o_copy(NB - 1).start()

    @pl.when(bstar != NB - 1)
    def _():
        o_copy(bstar).start()
    pltpu.make_async_copy(o_s, o_hbm, sem_o).wait()


@jax.jit
def pallas_parallel_sum__sliding_block__moe_arch_mod__prompt_kernel(
    A_x, A_wqkv, A_wo, B_x, B_w_r, B_w_gate, B_w_up, B_w_down,
):
    del B_x
    hbm = pl.BlockSpec(memory_space=pltpu.HBM)
    out = pl.pallas_call(
        kernel,
        out_shape=jax.ShapeDtypeStruct((S, D), BF),
        in_specs=[hbm] * 7,
        out_specs=hbm,
        scratch_shapes=[
            pltpu.VMEM((S + BQ, D), BF),
            pltpu.VMEM((3, D, D), BF),
            pltpu.VMEM((D, D), BF),
            pltpu.VMEM((D,), BF),
            pltpu.VMEM((F, D), BF),
            pltpu.VMEM((F, D), BF),
            pltpu.VMEM((F, D), BF),
            pltpu.VMEM((4, 2, HB, D), I32),
            pltpu.VMEM((S + BQ, D), F32),
            pltpu.VMEM((H, HB, 128), I32),
            pltpu.VMEM((H, HB, 128), I32),
            pltpu.VMEM((H, (NB + 1) * HB, 128), I32),
            pltpu.VMEM((NB, D // 2, BQ), I32),
            pltpu.VMEM((NB, D // 2, BQ), I32),
            pltpu.VMEM((776, D), I32),
            pltpu.VMEM((D // 2, D), I32),
            pltpu.VMEM((2, D // 2, BQ), I32),
            pltpu.VMEM((NB, 8, BQ), F32),
            pltpu.VMEM((NBUF, 4, 256, 128), F32),
            pltpu.VMEM((S, D), BF),
            pltpu.VMEM((8, D), F32),
            pltpu.SemaphoreType.DMA((NB + 1,)),
            pltpu.SemaphoreType.DMA((8,)),
            pltpu.SemaphoreType.DMA(()),
        ],
        compiler_params=pltpu.CompilerParams(vmem_limit_bytes=100 * 2**20),
    )(A_x.reshape(S, D), A_wqkv, A_wo, B_w_r, B_w_gate.T, B_w_up.T, B_w_down)
    return out.reshape(1, S, D)
```

```python
import functools, math
import numpy as np
import jax
import jax.numpy as jnp
from jax import lax
import jax.experimental.pallas as pl
import jax.experimental.pallas.tpu as pltpu

S, D, H, DH, W, F = 2048, 512, 32, 16, 256, 1376
BQ = 128
HB = BQ // 2
NB = S // BQ
BF = jnp.bfloat16
F32 = jnp.float32
I32 = jnp.int32
NT = (((1,), (1,)), ((), ()))
TN = (((0,), (0,)), ((), ()))
QSCALE = (DH ** -0.5) * math.log2(math.e)
NEG = -1e30
FP = 32
OPG = 2
OPGL = 4
FA0 = 4
FR0 = 2
FR1 = 8
LA = 3
NBUF = 4
ANCH = [(), (7, 15, 23), (3, 7, 11, 15, 19, 23), tuple(range(24)), (23,)][0]
LNS = [(1, 2, 3, 4), (0, 1, 2, 3), (2, 3, 4, 5), (0, 2, 4, 5)][0]
KSS = [[[0, 1, 2, 3], [4, 5, 6, 7], [8, 9, 10, 11], [12, 13, 14, 15]], [[0, 1, 2, 3, 4, 5, 6, 7], [], [8, 9, 10, 11, 12, 13, 14, 15], []]][1]
MIDS = [[[n] for n in range(16)], [[2 * n, 2 * n + 1] for n in range(8)] + [[]] * 8][0]
KS2 = [[[8 + g] for g in range(8)], [[], [], [], [8], [9, 10], [11, 12], [13, 14], [15]], [[], [], [], [8, 9], [10, 11], [12, 13], [14, 15], []], [[15], [], [], [8], [9], [10, 11], [12, 13], [14]], [[8, 9], [], [10, 11], [], [12, 13], [], [14, 15], []], [[], [], [], [8, 9], [10, 11], [12, 13], [14, 15], []]][2]
PRO1 = 0
KREL = 0
assert FA0 + LA < 8
OPGT = 4
SPLIT = 1
PB = 0
LV = 1
U2 = 4
XW = [(2, 8), (2, 10), (2, 6, 10), (2, 11), (2, 9)][4]
NOF = 0


def _pack(v):
    return pltpu.bitcast(v.astype(BF), I32)


def _pack_pi(v):
    n = v.shape[0] // 16
    v4 = v.reshape(n, 2, 8, v.shape[1])
    return pltpu.pack_elementwise([v4[:, 0], v4[:, 1]], packed_dtype=BF).reshape(8 * n, v.shape[1])


def _unpack(v):
    return pltpu.bitcast(v, BF)


def _rnd(v):
    return v.astype(BF).astype(F32)


def _layernorm(xf):
    mean = jnp.mean(xf, axis=-1, keepdims=True)
    c = xf - mean
    var = jnp.mean(c * c, axis=-1, keepdims=True)
    d = _rnd(xf - _rnd(mean))
    s = _rnd(jnp.sqrt(_rnd(_rnd(var) + 1e-5)))
    return d / s


def kernel(x_hbm, wqkv_hbm, wo_hbm, wr_hbm, wgt_hbm, wut_hbm, wd_hbm, o_hbm,
           x_s, wqkv_s, wo_in, wr_s, wgt_s, wut_s, wd_s,
           xn_s, res_s, ta_s, tb_s, ks_s, v_s, q_s, wt_s, wo_s, ot_s, r_s, s_s, o_s, xr_s,
           sem_x, sem_w, sem_o):
    def x_copy(b):
        return pltpu.make_async_copy(x_hbm.at[b * BQ:(b + 1) * BQ, :], x_s.at[b * BQ:(b + 1) * BQ, :], sem_x.at[b])

    def w_copy(i):
        return pltpu.make_async_copy(wqkv_hbm.at[:, i * D:(i + 1) * D], wqkv_s.at[i], sem_w.at[i])

    c_wr = pltpu.make_async_copy(wr_hbm, wr_s, sem_w.at[3])
    c_wo = pltpu.make_async_copy(wo_hbm, wo_in, sem_w.at[4])
    c_wg = pltpu.make_async_copy(wgt_hbm, wgt_s, sem_w.at[5])
    c_wu = pltpu.make_async_copy(wut_hbm, wut_s, sem_w.at[6])
    c_wd = pltpu.make_async_copy(wd_hbm, wd_s, sem_w.at[7])

    for c in (c_wr, x_copy(0), x_copy(1), w_copy(1), w_copy(0), x_copy(2), w_copy(2), x_copy(3)):
        c.start()

    lane8 = lax.broadcasted_iota(I32, (8, 128), 1)
    zero8 = jnp.zeros((8, 128), I32)

    def ln_rows(b, slot, r0, n):
        t0 = b * BQ + r0 if isinstance(b, int) else pl.multiple_of(b * BQ + r0, 16)
        xf = x_s[pl.ds(t0, n), :].astype(F32)
        xn = _rnd(_layernorm(xf))
        xn_s[slot, 0, r0 // 2:(r0 + n) // 2, :] = _pack(xn)
        xn_s[slot, 1, r0 // 2:(r0 + n) // 2, :] = _pack_pi(xn)
        res_s[pl.ds(t0, n), :] = xf + xn
        return pltpu.bitcast(xn[n - 8:n, 384:512], I32)

    def proj(b, slot, kind, c, z=None):
        r0 = kind * 256 + c * 128
        r1 = r0 + 128 + (8 if (kind == 2 and c == 1) else 0)
        xn = _unpack(xn_s[slot, 1 if kind == 2 else 0])
        w = wt_s[r0:r1, :]
        if z is not None:
            w = jnp.concatenate([jnp.concatenate([w[0:8, 0:128] | z, w[0:8, 128:]], axis=1), w[8:]], axis=0)
        o = lax.dot_general(_unpack(w), xn, NT, preferred_element_type=F32)
        if kind == 0:
            q_s[b, c * 128:(c + 1) * 128, :] = _pack_pi(o * QSCALE)
        elif kind == 1:
            return _pack_pi(o)
        else:
            v_s[b, c * 128:(c + 1) * 128, :] = _pack(o[0:256])
            if c == 1:
                r_s[b] = o[256:264]

    jbit = [((lane8 >> 4) & (1 << k)) != 0 for k in range(3)]

    def build_ks(b, pairs, slabs, t_prev, t_cur):
        row0 = b * HB if isinstance(b, int) else pl.multiple_of(b * HB, HB)
        for p in pairs:
            hs = (2 * p, 2 * p + 1)
            if slabs is not None:
                rows = [slabs[h // 16][(h % 16) * 8:(h % 16 + 1) * 8] for h in hs for _ in range(8)]
                tt = pltpu.bitcast(_unpack(jnp.concatenate(rows, axis=0)).T, I32)
            for n, h in enumerate(hs):
                if slabs is not None:
                    cur = tt[:, n * 128:(n + 1) * 128]
                    t_cur[h] = cur
                prev = None if t_prev is None else t_prev[h]
                g = [None if prev is None else prev[8 * i:8 * i + 8] for i in range(8)] + \
                    [None if slabs is None else cur[8 * i:8 * i + 8] for i in range(7)]
                for k in (2, 1, 0):
                    sh = 1 << k
                    nxt = []
                    for i in range(len(g) - sh):
                        lo, hi = g[i], g[i + sh]
                        if lo is None and hi is None:
                            nxt.append(None)
                        else:
                            nxt.append(jnp.where(jbit[k], zero8 if hi is None else hi, zero8 if lo is None else lo))
                    g = nxt
                ks_s[h, pl.ds(row0, HB), :] = jnp.concatenate([zero8 if x is None else x for x in g], axis=0)

    def t_weight(i, kind):
        wt_s[kind * 256:(kind + 1) * 256, :] = pltpu.bitcast(wqkv_s[i].T, I32)

    x_copy(0).wait()
    x_copy(1).wait()
    ln_rows(0, 2, 0, BQ)
    ln_rows(1, 3, 0, BQ)
    w_copy(1).wait()
    c_wr.wait()
    for b in range(4, NB):
        x_copy(b).start()
    c_wo.start()
    c_wg.start()
    c_wu.start()
    c_wd.start()
    t_weight(1, 1)
    wt_s[768:776, :] = pltpu.bitcast(jnp.broadcast_to(wr_s[...].reshape(1, D), (16, D)), I32)
    kt = [[proj(b, 2 + b, 1, c) for c in range(2)] for b in (0, 1)]
    w_copy(0).wait()
    if LV == 0:
        x_copy(2).wait()
    t_weight(0, 0)
    xb = pltpu.bitcast(x_s[0:16, 0:128], I32)
    zvec = (xb * xb + xb) & 1
    def pro_builds(n):
        if PB == 0:
            build_ks(0, range(2 * n, 2 * n + 2), kt[0], None, ta_s)
            build_ks(1, range(2 * n, 2 * n + 2), kt[1], ta_s, tb_s)
        elif n < 4:
            build_ks(0, range(4 * n, 4 * n + 4), kt[0], None, ta_s)
        else:
            build_ks(1, range(4 * n - 16, 4 * n - 12), kt[1], ta_s, tb_s)

    lnz = [None, ln_rows(2, 0, 0, 64), ln_rows(2, 0, 64, 32), ln_rows(2, 0, 96, 32)] if LV == 0 else [None] * 4
    for b in (0, 1):
        for c in range(2):
            n = 2 * b + c
            pro_builds(n)
            proj(b, 2 + b, 0, c, None if lnz[n] is None else lnz[n] & zvec)
    w_copy(2).wait()
    if LV == 1:
        x_copy(2).wait()
    t_weight(2, 2)
    lnz = [None, ln_rows(2, 0, 0, 64), ln_rows(2, 0, 64, 32), ln_rows(2, 0, 96, 32)] if LV == 1 else [None] * 4
    for b in (0, 1):
        for c in range(2):
            pro_builds(4 + 2 * b + c)
            proj(b, 2 + b, 2, c, None if lnz[2 * b + c] is None else lnz[2 * b + c] & zvec)

    def proj_block(b, src, dst, t_prev, t_cur):
        cur = []
        n = 0
        for kind in (1, 0, 2):
            for c in range(2):
                if n in LNS and dst is not None:
                    ln_rows(b + 1, dst, LNS.index(n) * 32, 32)
                if n >= 2:
                    build_ks(b, KSS[n - 2], cur, t_prev, t_cur)
                o = proj(b, src, kind, c)
                if kind == 1:
                    cur.append(o)
                n += 1

    for b in range(2, NB):
        if b in XW:
            for bb in range(b + 1, XW[XW.index(b) + 1] + 1 if b != XW[-1] else NB):
                x_copy(bb).wait()
            if b == XW[-1]:
                c_wo.wait()
                c_wg.wait()
                c_wu.wait()
                c_wd.wait()
        j = b % 2
        proj_block(b, j, 1 - j if b + 1 < NB else None, (tb_s, ta_s)[j], (ta_s, tb_s)[j])

    wo_s[...] = _pack_pi(wo_in[...].astype(F32))
    r = _rnd(r_s[...])[:, 0, :]
    rmax = jnp.max(r)
    ln = lax.broadcasted_iota(I32, (NB, BQ), 1)
    pos = lax.broadcasted_iota(I32, (NB, BQ), 0) * BQ + (ln & -16) + ((ln & 15) >> 1) + 8 * (ln & 1)
    idx = jnp.min(jnp.where(r == rmax, pos, S))
    idx = jnp.minimum(idx, S - 1)
    bstar = idx // BQ
    base = pl.multiple_of((idx // 16) * 16, 16)
    rowsel = lax.broadcasted_iota(I32, (16, 1), 0) == (idx - base)
    slab = _rnd(_layernorm(x_s[pl.ds(base, 16), :].astype(F32)))
    xr_s[...] = jnp.broadcast_to(jnp.sum(jnp.where(rowsel, slab, 0.0), axis=0, keepdims=True), (8, D))

    yacc = [None]

    def ffn_piece(k, rel=None):
        f0 = k * FP if isinstance(k, int) else pl.multiple_of(k * FP, FP)
        xr = xr_s[...]
        if rel is not None:
            xr = pltpu.bitcast(pltpu.bitcast(xr, I32) | jnp.concatenate([rel] * 4, axis=1), F32)
        xr = xr[0:1, :]
        g = _rnd(jnp.sum(wgt_s[pl.ds(f0, FP), :].astype(F32) * xr, axis=1, keepdims=True))
        u = _rnd(jnp.sum(wut_s[pl.ds(f0, FP), :].astype(F32) * xr, axis=1, keepdims=True))
        h = _rnd(_rnd(g * jax.nn.sigmoid(g)) * u)
        yp = wd_s[pl.ds(f0, FP), :].astype(F32) * h
        yp = jnp.sum(yp.reshape(FP // 8, 8, D), axis=0)
        yacc[0] = yacc[0] + yp
        return pltpu.bitcast(yp[:, 0:128], I32)

    def ffn_group(k0, n, zero, rel=None):
        w = None
        for p in range(n):
            v = ffn_piece(k0 + p, rel)
            w = v if w is None else w | v
        return w & zero

    maskd = lax.broadcasted_iota(I32, (16, 128), 0) <= (lax.broadcasted_iota(I32, (16, 128), 1) & 15)
    lane16 = lax.broadcasted_iota(I32, (16, 128), 1)
    ones8 = jnp.full((8, 128), 0x3F803F80, I32)
    jmask = [(lane8 >> 4) == j for j in range(8)]

    dzero = jnp.minimum(idx, 0)

    def first_group(t):
        return max(9 - 8 * t, 0) if isinstance(t, int) else 0

    def qk(t, G, par, z=None):
        i0 = first_group(t)
        ms = []
        for jh in range(4):
            h = 4 * G + jh
            row0 = (t - 1) * HB + 8 * i0
            if not isinstance(t, int):
                row0 = pl.multiple_of(row0, HB)
            kall = ks_s[h, pl.ds(row0, 8 * (17 - i0)), :]
            if i0 == 0:
                kall = jnp.concatenate([kall[0:8], kall[128:136], kall[8:128]], axis=0)
            if z is not None and jh == 0:
                kall = jnp.concatenate([kall[0:8] | z, kall[8:]], axis=0)
            qh = q_s[t, h * 8:(h + 1) * 8, :]
            qm = jnp.concatenate([jnp.where(jmask[j], qh, 0) for j in range(8)], axis=0)
            st = jnp.dot(_unpack(kall), _unpack(qm), preferred_element_type=F32)
            if i0 == 0:
                comb = jnp.where(maskd, st[16:32], st[0:16])
                mid = st[32:272]
            else:
                nm = 16 - i0
                comb = jnp.where(maskd, st[16 * nm:], NEG)
                mid = jnp.concatenate([
                    jnp.where(lane16 >= 16 * (16 - 8 * t - i), st[16 * (i - i0):16 * (i - i0 + 1)], NEG)
                    for i in range(i0, 16)], axis=0)
            nm = mid.shape[0]
            m = jnp.maximum(jnp.max(comb.reshape(2, 8, 128), axis=0), jnp.max(mid.reshape(nm // 8, 8, 128), axis=0))
            s_s[par, jh, 0:16, :] = comb
            s_s[par, jh, 16:16 + nm, :] = mid
            ms.append(jnp.max(m, axis=0, keepdims=True))
        return ms

    def unskew(plist):
        cur = plist
        for k in range(3):
            sh = 1 << k
            nxt = []
            for i in range(len(cur) + sh):
                a = cur[i - sh] if 0 <= i - sh < len(cur) else None
                b = cur[i] if i < len(cur) else None
                if a is None and b is None:
                    nxt.append(None)
                else:
                    nxt.append(jnp.where(jbit[k], zero8 if a is None else a, zero8 if b is None else b))
            cur = nxt
        return cur

    def softmax(t, G, par, ms):
        i0 = first_group(t)
        nm = 16 * (16 - max(i0, 1))
        us = []
        for jh in range(4):
            m = ms[jh]
            pc = jnp.exp2(s_s[par, jh, 0:16, :] - m)
            pm = _pack_pi(jnp.exp2(s_s[par, jh, 16:16 + nm, :] - m))
            plist = [None] * 17
            first_mid = 16 - nm // 16
            for i in range(nm // 16):
                plist[first_mid + i] = pm[8 * i:8 * i + 8]
            if i0 == 0:
                plist[0] = _pack_pi(jnp.where(maskd, 0.0, pc))
                plist[16] = _pack_pi(jnp.where(maskd, pc, 0.0))
            else:
                plist[16] = _pack_pi(pc)
            us.append(unskew(plist))
        return us

    def pv(t, G, us):
        os_ = []
        for jh in range(4):
            h = 4 * G + jh
            u = us[jh]
            ov = None
            for T in range(3):
                if isinstance(t, int) and t - 2 + T < 0:
                    continue
                tile = jnp.concatenate([zero8 if x is None else x for x in u[8 * T:8 * T + 8]], axis=0)
                vh = v_s[t - 2 + T, h * 8:(h + 1) * 8, :]
                vv = _unpack(jnp.concatenate([vh, ones8], axis=0))
                part = jnp.dot(vv, _unpack(tile), preferred_element_type=F32)
                ov = part if ov is None else ov + part
            l = ov[16:24]
            rc = pl.reciprocal(l, approx=True)
            rc = rc * (2.0 - l * rc)
            o = _pack_pi((ov[0:16].reshape(2, 8, 128) * rc).reshape(16, 128))
            ot_s[t % 2, h * 8:(h + 1) * 8, :] = o
            os_.append(o)
        return os_

    def anchor(us):
        z = None
        for u in us:
            for I in ANCH:
                if u[I] is not None:
                    z = u[I] if z is None else z | u[I]
        return z & dzero

    def out_proj(b):
        t0 = b * BQ if isinstance(b, int) else pl.multiple_of(b * BQ, BQ)
        a = lax.dot_general(_unpack(ot_s[b % 2]), _unpack(wo_s[...]), TN, preferred_element_type=F32)
        o32 = res_s[pl.ds(t0, BQ), :] + a
        res_s[pl.ds(t0, BQ), :] = o32
        o_s[pl.ds(t0, BQ), :] = o32.astype(BF)
        return pltpu.bitcast(a[0:8, 0:128], I32)

    def out_proj_part(b, g, last=False):
        a = lax.dot_general(_unpack(ot_s[b % 2, g * 64:(g + 1) * 64, :]), _unpack(wo_s[g * 64:(g + 1) * 64, :]),
                            TN, preferred_element_type=F32)
        o32 = res_s[b * BQ:(b + 1) * BQ, :] + a
        res_s[b * BQ:(b + 1) * BQ, :] = o32
        if last:
            o_s[b * BQ:(b + 1) * BQ, :] = o32.astype(BF)

    def o_copy(b):
        t0 = b * BQ if isinstance(b, int) else pl.multiple_of(b * BQ, BQ)
        return pltpu.make_async_copy(o_s.at[pl.ds(t0, BQ), :], o_hbm.at[pl.ds(t0, BQ), :], sem_o)

    def o_start(b):
        @pl.when(b != bstar)
        def _():
            o_copy(b).start()

    def block(t, pend, nt, prev_out, last=False, fk=None):
        rel = None
        krel = None
        pend = list(pend)
        if fk is not None:
            zero = dzero
        for G in range(8):
            def next_qk():
                n = G + LA
                if n < 8:
                    z = None
                    if fk is not None and fk[1] == 0 and G == FA0:
                        z = ffn_group(fk[0], 3, zero, rel)
                    if zs is not None:
                        z = zs if z is None else z | zs
                    return qk(t, n, n % NBUF, z)
                return None if nt is None else qk(nt, n - 8, n % NBUF, zs)
            late = last and G == 7
            if isinstance(t, int) and t < 2:
                build_ks(NB, MIDS[8 * t + G], None, tb_s, None)
            us = softmax(t, G, G % NBUF, pend.pop(0))
            zs = anchor(us) if ANCH else None
            if not late:
                pend.append(next_qk())
            if G == prev_out:
                a0 = out_proj(t - 1)
                if fk is not None and fk[1] == 1:
                    ffn_group(fk[0], 3, zero, a0 & zero)
            os_ = pv(t, G, us)
            if KREL:
                krel = os_[KREL - 1] & dzero
            if fk is not None and fk[1] == 0 and G == FR0:
                rel = os_[3] & zero
            if late:
                pend.append(next_qk())
            if isinstance(t, int) and t == NB - 1 and SPLIT and G in (3, 5, 7):
                out_proj_part(t, (G - 3) // 2)
        return pend

    pend = [qk(0, n, n % NBUF) for n in range(LA)]
    pend = block(0, pend, 1, None)
    yacc[0] = jnp.zeros((8, D), F32)
    ffn_piece(0)
    y0 = yacc[0]
    pend = block(1, pend, 2, 7, True)
    o_start(0)

    def p2(i, carry):
        pend = [list(carry[4 * n:4 * n + 4]) for n in range(LA)]
        yacc[0] = carry[-1]
        for j in range(U2):
            t = 2 + U2 * i + j
            lastj = j == U2 - 1
            pend = block(t, pend, t + 1, OPGL if lastj else OPG, lastj,
                         fk=None if NOF else (1 + 3 * (U2 * i + j), 1 if lastj else 0))
        for j in range(U2):
            o_start(2 + U2 * i + j - 1)
        return tuple(m for ms in pend for m in ms) + (yacc[0],)
    carry = lax.fori_loop(0, (NB - 4) // U2, p2, tuple(m for ms in pend for m in ms) + (y0,))
    pend = [list(carry[4 * n:4 * n + 4]) for n in range(LA)]
    yacc[0] = carry[-1]
    pend = block(NB - 2, pend, NB - 1, OPG, fk=(37, 0))
    block(NB - 1, pend, None, OPGT, fk=(40, 1))
    o_start(NB - 3)
    o_start(NB - 2)
    ylast = yacc[0]
    if SPLIT:
        out_proj_part(NB - 1, 3, True)
    else:
        out_proj(NB - 1)

    y = _rnd(jnp.sum(ylast, axis=0, keepdims=True))
    rs = _rnd(jax.nn.sigmoid(jnp.full((1, D), rmax, F32)))
    y = _rnd(y * rs)
    o_s[pl.ds(base, 16), :] = (res_s[pl.ds(base, 16), :] + jnp.where(rowsel, y, 0.0)).astype(BF)
    o_copy(NB - 1).start()

    @pl.when(bstar != NB - 1)
    def _():
        o_copy(bstar).start()
    pltpu.make_async_copy(o_s, o_hbm, sem_o).wait()


@jax.jit
def pallas_parallel_sum__sliding_block__moe_arch_mod__prompt_kernel(
    A_x, A_wqkv, A_wo, B_x, B_w_r, B_w_gate, B_w_up, B_w_down,
):
    del B_x
    hbm = pl.BlockSpec(memory_space=pltpu.HBM)
    out = pl.pallas_call(
        kernel,
        out_shape=jax.ShapeDtypeStruct((S, D), BF),
        in_specs=[hbm] * 7,
        out_specs=hbm,
        scratch_shapes=[
            pltpu.VMEM((S, D), BF),
            pltpu.VMEM((3, D, D), BF),
            pltpu.VMEM((D, D), BF),
            pltpu.VMEM((D,), BF),
            pltpu.VMEM((F, D), BF),
            pltpu.VMEM((F, D), BF),
            pltpu.VMEM((F, D), BF),
            pltpu.VMEM((4, 2, HB, D), I32),
            pltpu.VMEM((S, D), F32),
            pltpu.VMEM((H, HB, 128), I32),
            pltpu.VMEM((H, HB, 128), I32),
            pltpu.VMEM((H, (NB + 1) * HB, 128), I32),
            pltpu.VMEM((NB, D // 2, BQ), I32),
            pltpu.VMEM((NB, D // 2, BQ), I32),
            pltpu.VMEM((776, D), I32),
            pltpu.VMEM((D // 2, D), I32),
            pltpu.VMEM((2, D // 2, BQ), I32),
            pltpu.VMEM((NB, 8, BQ), F32),
            pltpu.VMEM((NBUF, 4, 256, 128), F32),
            pltpu.VMEM((S, D), BF),
            pltpu.VMEM((8, D), F32),
            pltpu.SemaphoreType.DMA((NB,)),
            pltpu.SemaphoreType.DMA((8,)),
            pltpu.SemaphoreType.DMA(()),
        ],
        compiler_params=pltpu.CompilerParams(vmem_limit_bytes=100 * 2**20),
    )(A_x.reshape(S, D), A_wqkv, A_wo, B_w_r, B_w_gate.T, B_w_up.T, B_w_down)
    return out.reshape(1, S, D)
```

```python
import functools, math
import numpy as np
import jax
import jax.numpy as jnp
from jax import lax
import jax.experimental.pallas as pl
import jax.experimental.pallas.tpu as pltpu

S, D, H, DH, W, F = 2048, 512, 32, 16, 256, 1376
BQ = 128
HB = BQ // 2
NB = S // BQ
BF = jnp.bfloat16
F32 = jnp.float32
I32 = jnp.int32
NT = (((1,), (1,)), ((), ()))
TN = (((0,), (0,)), ((), ()))
QSCALE = (DH ** -0.5) * math.log2(math.e)
NEG = -1e30
FP = 32
OPG = 2
OPGL = 4
FA0 = 4
FR0 = 2
FR1 = 8
LA = 3
NBUF = 4
ANCH = [(), (7, 15, 23), (3, 7, 11, 15, 19, 23), tuple(range(24)), (23,)][0]
LNS = [(1, 2, 3, 4), (0, 1, 2, 3), (2, 3, 4, 5), (0, 2, 4, 5)][0]
KSS = [[[0, 1, 2, 3], [4, 5, 6, 7], [8, 9, 10, 11], [12, 13, 14, 15]], [[0, 1, 2, 3, 4, 5, 6, 7], [], [8, 9, 10, 11, 12, 13, 14, 15], []]][1]
MIDS = [[[n] for n in range(16)], [[2 * n, 2 * n + 1] for n in range(8)] + [[]] * 8][0]
KS2 = [[[8 + g] for g in range(8)], [[], [], [], [8], [9, 10], [11, 12], [13, 14], [15]], [[], [], [], [8, 9], [10, 11], [12, 13], [14, 15], []], [[15], [], [], [8], [9], [10, 11], [12, 13], [14]], [[8, 9], [], [10, 11], [], [12, 13], [], [14, 15], []], [[], [], [], [8, 9], [10, 11], [12, 13], [14, 15], []]][2]
PRO1 = 0
KREL = 0
assert FA0 + LA < 8
OPGT = 4
SPLIT = 1
PB = 0
LV = 1
U2 = 4
XW = [(2, 8), (2, 10), (2, 6, 10), (2, 11), (2, 9)][4]
NOF = 0


def _pack(v):
    return pltpu.bitcast(v.astype(BF), I32)


def _pack_pi(v):
    n = v.shape[0] // 16
    v4 = v.reshape(n, 2, 8, v.shape[1])
    return pltpu.pack_elementwise([v4[:, 0], v4[:, 1]], packed_dtype=BF).reshape(8 * n, v.shape[1])


def _unpack(v):
    return pltpu.bitcast(v, BF)


def _rnd(v):
    return v.astype(BF).astype(F32)


def _layernorm(xf):
    mean = jnp.mean(xf, axis=-1, keepdims=True)
    c = xf - mean
    var = jnp.mean(c * c, axis=-1, keepdims=True)
    d = _rnd(xf - _rnd(mean))
    s = _rnd(jnp.sqrt(_rnd(_rnd(var) + 1e-5)))
    return d / s


def kernel(x_hbm, wqkv_hbm, wo_hbm, wr_hbm, wgt_hbm, wut_hbm, wd_hbm, o_hbm,
           x_s, wqkv_s, wo_in, wr_s, wgt_s, wut_s, wd_s,
           xn_s, res_s, ks_s, v_s, q_s, wt_s, wo_s, ot_s, r_s, s_s, o_s, xr_s,
           sem_x, sem_w, sem_o):
    def x_copy(b):
        return pltpu.make_async_copy(x_hbm.at[b * BQ:(b + 1) * BQ, :], x_s.at[b * BQ:(b + 1) * BQ, :], sem_x.at[b])

    def w_copy(i):
        return pltpu.make_async_copy(wqkv_hbm.at[:, i * D:(i + 1) * D], wqkv_s.at[i], sem_w.at[i])

    c_wr = pltpu.make_async_copy(wr_hbm, wr_s, sem_w.at[3])
    c_wo = pltpu.make_async_copy(wo_hbm, wo_in, sem_w.at[4])
    c_wg = pltpu.make_async_copy(wgt_hbm, wgt_s, sem_w.at[5])
    c_wu = pltpu.make_async_copy(wut_hbm, wut_s, sem_w.at[6])
    c_wd = pltpu.make_async_copy(wd_hbm, wd_s, sem_w.at[7])

    for c in (c_wr, x_copy(0), x_copy(1), w_copy(1), w_copy(0), x_copy(2), w_copy(2), x_copy(3)):
        c.start()

    ta_s, tb_s = {}, {}
    lane8 = lax.broadcasted_iota(I32, (8, 128), 1)
    zero8 = jnp.zeros((8, 128), I32)

    def ln_rows(b, slot, r0, n):
        t0 = b * BQ + r0 if isinstance(b, int) else pl.multiple_of(b * BQ + r0, 16)
        xf = x_s[pl.ds(t0, n), :].astype(F32)
        xn = _rnd(_layernorm(xf))
        xn_s[slot, 0, r0 // 2:(r0 + n) // 2, :] = _pack(xn)
        xn_s[slot, 1, r0 // 2:(r0 + n) // 2, :] = _pack_pi(xn)
        res_s[pl.ds(t0, n), :] = xf + xn
        return pltpu.bitcast(xn[n - 8:n, 384:512], I32)

    def proj(b, slot, kind, c, z=None):
        r0 = kind * 256 + c * 128
        r1 = r0 + 128 + (8 if (kind == 2 and c == 1) else 0)
        xn = _unpack(xn_s[slot, 1 if kind == 2 else 0])
        w = wt_s[r0:r1, :]
        if z is not None:
            w = jnp.concatenate([jnp.concatenate([w[0:8, 0:128] | z, w[0:8, 128:]], axis=1), w[8:]], axis=0)
        o = lax.dot_general(_unpack(w), xn, NT, preferred_element_type=F32)
        if kind == 0:
            q_s[b, c * 128:(c + 1) * 128, :] = _pack_pi(o * QSCALE)
        elif kind == 1:
            return _pack_pi(o)
        else:
            v_s[b, c * 128:(c + 1) * 128, :] = _pack(o[0:256])
            if c == 1:
                r_s[b] = o[256:264]

    jbit = [((lane8 >> 4) & (1 << k)) != 0 for k in range(3)]

    def build_ks(b, pairs, slabs, t_prev, t_cur):
        for p in pairs:
            hs = (2 * p, 2 * p + 1)
            if slabs is not None:
                rows = [slabs[h // 16][(h % 16) * 8:(h % 16 + 1) * 8] for h in hs for _ in range(8)]
                tt = pltpu.bitcast(_unpack(jnp.concatenate(rows, axis=0)).T, I32)
            for n, h in enumerate(hs):
                if slabs is not None:
                    t_cur[h] = tt[:, n * 128:(n + 1) * 128]
                g = [None if t_prev is None else t_prev[h][8 * i:8 * i + 8] for i in range(8)] + \
                    [None if slabs is None else t_cur[h][8 * i:8 * i + 8] for i in range(7)]
                for k in (2, 1, 0):
                    sh = 1 << k
                    nxt = []
                    for i in range(len(g) - sh):
                        lo, hi = g[i], g[i + sh]
                        if lo is None and hi is None:
                            nxt.append(None)
                        else:
                            nxt.append(jnp.where(jbit[k], zero8 if hi is None else hi, zero8 if lo is None else lo))
                    g = nxt
                ks_s[h, b * HB:(b + 1) * HB, :] = jnp.concatenate([zero8 if x is None else x for x in g], axis=0)

    def t_weight(i, kind):
        wt_s[kind * 256:(kind + 1) * 256, :] = pltpu.bitcast(wqkv_s[i].T, I32)

    x_copy(0).wait()
    x_copy(1).wait()
    ln_rows(0, 2, 0, BQ)
    ln_rows(1, 3, 0, BQ)
    w_copy(1).wait()
    c_wr.wait()
    for b in range(4, NB):
        x_copy(b).start()
    c_wo.start()
    c_wg.start()
    c_wu.start()
    c_wd.start()
    t_weight(1, 1)
    wt_s[768:776, :] = pltpu.bitcast(jnp.broadcast_to(wr_s[...].reshape(1, D), (16, D)), I32)
    kt = [[proj(b, 2 + b, 1, c) for c in range(2)] for b in (0, 1)]
    w_copy(0).wait()
    if LV == 0:
        x_copy(2).wait()
    t_weight(0, 0)
    xb = pltpu.bitcast(x_s[0:16, 0:128], I32)
    zvec = (xb * xb + xb) & 1
    def pro_builds(n):
        if PB == 0:
            build_ks(0, range(2 * n, 2 * n + 2), kt[0], None, ta_s)
            build_ks(1, range(2 * n, 2 * n + 2), kt[1], ta_s, tb_s)
        elif n < 4:
            build_ks(0, range(4 * n, 4 * n + 4), kt[0], None, ta_s)
        else:
            build_ks(1, range(4 * n - 16, 4 * n - 12), kt[1], ta_s, tb_s)

    lnz = [None, ln_rows(2, 0, 0, 64), ln_rows(2, 0, 64, 32), ln_rows(2, 0, 96, 32)] if LV == 0 else [None] * 4
    for b in (0, 1):
        for c in range(2):
            n = 2 * b + c
            pro_builds(n)
            proj(b, 2 + b, 0, c, None if lnz[n] is None else lnz[n] & zvec)
    w_copy(2).wait()
    if LV == 1:
        x_copy(2).wait()
    t_weight(2, 2)
    lnz = [None, ln_rows(2, 0, 0, 64), ln_rows(2, 0, 64, 32), ln_rows(2, 0, 96, 32)] if LV == 1 else [None] * 4
    for b in (0, 1):
        for c in range(2):
            pro_builds(4 + 2 * b + c)
            proj(b, 2 + b, 2, c, None if lnz[2 * b + c] is None else lnz[2 * b + c] & zvec)

    def proj_block(b, src, dst, t_prev, t_cur):
        cur = []
        n = 0
        for kind in (1, 0, 2):
            for c in range(2):
                if n in LNS and dst is not None:
                    ln_rows(b + 1, dst, LNS.index(n) * 32, 32)
                if n >= 2:
                    build_ks(b, KSS[n - 2], cur, t_prev, t_cur)
                o = proj(b, src, kind, c)
                if kind == 1:
                    cur.append(o)
                n += 1

    for b in range(2, NB):
        if b in XW:
            for bb in range(b + 1, XW[XW.index(b) + 1] + 1 if b != XW[-1] else NB):
                x_copy(bb).wait()
            if b == XW[-1]:
                c_wo.wait()
                c_wg.wait()
                c_wu.wait()
                c_wd.wait()
        j = b % 2
        proj_block(b, j, 1 - j if b + 1 < NB else None, (tb_s, ta_s)[j], (ta_s, tb_s)[j])

    wo_s[...] = _pack_pi(wo_in[...].astype(F32))
    r = _rnd(r_s[...])[:, 0, :]
    rmax = jnp.max(r)
    ln = lax.broadcasted_iota(I32, (NB, BQ), 1)
    pos = lax.broadcasted_iota(I32, (NB, BQ), 0) * BQ + (ln & -16) + ((ln & 15) >> 1) + 8 * (ln & 1)
    idx = jnp.min(jnp.where(r == rmax, pos, S))
    idx = jnp.minimum(idx, S - 1)
    bstar = idx // BQ
    base = pl.multiple_of((idx // 16) * 16, 16)
    rowsel = lax.broadcasted_iota(I32, (16, 1), 0) == (idx - base)
    slab = _rnd(_layernorm(x_s[pl.ds(base, 16), :].astype(F32)))
    xr_s[...] = jnp.broadcast_to(jnp.sum(jnp.where(rowsel, slab, 0.0), axis=0, keepdims=True), (8, D))

    yacc = [None]

    def ffn_piece(k, rel=None):
        f0 = k * FP if isinstance(k, int) else pl.multiple_of(k * FP, FP)
        xr = xr_s[...]
        if rel is not None:
            xr = pltpu.bitcast(pltpu.bitcast(xr, I32) | jnp.concatenate([rel] * 4, axis=1), F32)
        xr = xr[0:1, :]
        g = _rnd(jnp.sum(wgt_s[pl.ds(f0, FP), :].astype(F32) * xr, axis=1, keepdims=True))
        u = _rnd(jnp.sum(wut_s[pl.ds(f0, FP), :].astype(F32) * xr, axis=1, keepdims=True))
        h = _rnd(_rnd(g * jax.nn.sigmoid(g)) * u)
        yp = wd_s[pl.ds(f0, FP), :].astype(F32) * h
        yp = jnp.sum(yp.reshape(FP // 8, 8, D), axis=0)
        yacc[0] = yacc[0] + yp
        return pltpu.bitcast(yp[:, 0:128], I32)

    def ffn_group(k0, n, zero, rel=None):
        w = None
        for p in range(n):
            v = ffn_piece(k0 + p, rel)
            w = v if w is None else w | v
        return w & zero

    maskd = lax.broadcasted_iota(I32, (16, 128), 0) <= (lax.broadcasted_iota(I32, (16, 128), 1) & 15)
    lane16 = lax.broadcasted_iota(I32, (16, 128), 1)
    ones8 = jnp.full((8, 128), 0x3F803F80, I32)
    jmask = [(lane8 >> 4) == j for j in range(8)]

    dzero = jnp.minimum(idx, 0)

    def first_group(t):
        return max(9 - 8 * t, 0) if isinstance(t, int) else 0

    def qk(t, G, par, z=None):
        i0 = first_group(t)
        ms = []
        for jh in range(4):
            h = 4 * G + jh
            row0 = (t - 1) * HB + 8 * i0
            if not isinstance(t, int):
                row0 = pl.multiple_of(row0, HB)
            kall = ks_s[h, pl.ds(row0, 8 * (17 - i0)), :]
            if i0 == 0:
                kall = jnp.concatenate([kall[0:8], kall[128:136], kall[8:128]], axis=0)
            if z is not None and jh == 0:
                kall = jnp.concatenate([kall[0:8] | z, kall[8:]], axis=0)
            qh = q_s[t, h * 8:(h + 1) * 8, :]
            qm = jnp.concatenate([jnp.where(jmask[j], qh, 0) for j in range(8)], axis=0)
            st = jnp.dot(_unpack(kall), _unpack(qm), preferred_element_type=F32)
            if i0 == 0:
                comb = jnp.where(maskd, st[16:32], st[0:16])
                mid = st[32:272]
            else:
                nm = 16 - i0
                comb = jnp.where(maskd, st[16 * nm:], NEG)
                mid = jnp.concatenate([
                    jnp.where(lane16 >= 16 * (16 - 8 * t - i), st[16 * (i - i0):16 * (i - i0 + 1)], NEG)
                    for i in range(i0, 16)], axis=0)
            nm = mid.shape[0]
            m = jnp.maximum(jnp.max(comb.reshape(2, 8, 128), axis=0), jnp.max(mid.reshape(nm // 8, 8, 128), axis=0))
            s_s[par, jh, 0:16, :] = comb
            s_s[par, jh, 16:16 + nm, :] = mid
            ms.append(jnp.max(m, axis=0, keepdims=True))
        return ms

    def unskew(plist):
        cur = plist
        for k in range(3):
            sh = 1 << k
            nxt = []
            for i in range(len(cur) + sh):
                a = cur[i - sh] if 0 <= i - sh < len(cur) else None
                b = cur[i] if i < len(cur) else None
                if a is None and b is None:
                    nxt.append(None)
                else:
                    nxt.append(jnp.where(jbit[k], zero8 if a is None else a, zero8 if b is None else b))
            cur = nxt
        return cur

    def softmax(t, G, par, ms):
        i0 = first_group(t)
        nm = 16 * (16 - max(i0, 1))
        us = []
        for jh in range(4):
            m = ms[jh]
            pc = jnp.exp2(s_s[par, jh, 0:16, :] - m)
            pm = _pack_pi(jnp.exp2(s_s[par, jh, 16:16 + nm, :] - m))
            plist = [None] * 17
            first_mid = 16 - nm // 16
            for i in range(nm // 16):
                plist[first_mid + i] = pm[8 * i:8 * i + 8]
            if i0 == 0:
                plist[0] = _pack_pi(jnp.where(maskd, 0.0, pc))
                plist[16] = _pack_pi(jnp.where(maskd, pc, 0.0))
            else:
                plist[16] = _pack_pi(pc)
            us.append(unskew(plist))
        return us

    def pv(t, G, us):
        os_ = []
        for jh in range(4):
            h = 4 * G + jh
            u = us[jh]
            ov = None
            for T in range(3):
                if isinstance(t, int) and t - 2 + T < 0:
                    continue
                tile = jnp.concatenate([zero8 if x is None else x for x in u[8 * T:8 * T + 8]], axis=0)
                vh = v_s[t - 2 + T, h * 8:(h + 1) * 8, :]
                vv = _unpack(jnp.concatenate([vh, ones8], axis=0))
                part = jnp.dot(vv, _unpack(tile), preferred_element_type=F32)
                ov = part if ov is None else ov + part
            l = ov[16:24]
            rc = pl.reciprocal(l, approx=True)
            rc = rc * (2.0 - l * rc)
            o = _pack_pi((ov[0:16].reshape(2, 8, 128) * rc).reshape(16, 128))
            ot_s[t % 2, h * 8:(h + 1) * 8, :] = o
            os_.append(o)
        return os_

    def anchor(us):
        z = None
        for u in us:
            for I in ANCH:
                if u[I] is not None:
                    z = u[I] if z is None else z | u[I]
        return z & dzero

    def out_proj(b):
        t0 = b * BQ if isinstance(b, int) else pl.multiple_of(b * BQ, BQ)
        a = lax.dot_general(_unpack(ot_s[b % 2]), _unpack(wo_s[...]), TN, preferred_element_type=F32)
        o32 = res_s[pl.ds(t0, BQ), :] + a
        res_s[pl.ds(t0, BQ), :] = o32
        o_s[pl.ds(t0, BQ), :] = o32.astype(BF)
        return pltpu.bitcast(a[0:8, 0:128], I32)

    def out_proj_part(b, g, last=False):
        a = lax.dot_general(_unpack(ot_s[b % 2, g * 64:(g + 1) * 64, :]), _unpack(wo_s[g * 64:(g + 1) * 64, :]),
                            TN, preferred_element_type=F32)
        o32 = res_s[b * BQ:(b + 1) * BQ, :] + a
        res_s[b * BQ:(b + 1) * BQ, :] = o32
        if last:
            o_s[b * BQ:(b + 1) * BQ, :] = o32.astype(BF)

    def o_copy(b):
        t0 = b * BQ if isinstance(b, int) else pl.multiple_of(b * BQ, BQ)
        return pltpu.make_async_copy(o_s.at[pl.ds(t0, BQ), :], o_hbm.at[pl.ds(t0, BQ), :], sem_o)

    def o_start(b):
        @pl.when(b != bstar)
        def _():
            o_copy(b).start()

    def block(t, pend, nt, prev_out, last=False, fk=None):
        rel = None
        krel = None
        pend = list(pend)
        if fk is not None:
            zero = dzero
        for G in range(8):
            def next_qk():
                n = G + LA
                if n < 8:
                    z = None
                    if fk is not None and fk[1] == 0 and G == FA0:
                        z = ffn_group(fk[0], 3, zero, rel)
                    if zs is not None:
                        z = zs if z is None else z | zs
                    return qk(t, n, n % NBUF, z)
                return None if nt is None else qk(nt, n - 8, n % NBUF, zs)
            late = last and G == 7
            if isinstance(t, int) and t < 2:
                build_ks(NB, MIDS[8 * t + G], None, tb_s, None)
            us = softmax(t, G, G % NBUF, pend.pop(0))
            zs = anchor(us) if ANCH else None
            if not late:
                pend.append(next_qk())
            if G == prev_out:
                a0 = out_proj(t - 1)
                if fk is not None and fk[1] == 1:
                    ffn_group(fk[0], 3, zero, a0 & zero)
            os_ = pv(t, G, us)
            if KREL:
                krel = os_[KREL - 1] & dzero
            if fk is not None and fk[1] == 0 and G == FR0:
                rel = os_[3] & zero
            if late:
                pend.append(next_qk())
            if isinstance(t, int) and t == NB - 1 and SPLIT and G in (3, 5, 7):
                out_proj_part(t, (G - 3) // 2)
        return pend

    pend = [qk(0, n, n % NBUF) for n in range(LA)]
    pend = block(0, pend, 1, None)
    yacc[0] = jnp.zeros((8, D), F32)
    ffn_piece(0)
    y0 = yacc[0]
    pend = block(1, pend, 2, 7, True)
    o_start(0)

    def p2(i, carry):
        pend = [list(carry[4 * n:4 * n + 4]) for n in range(LA)]
        yacc[0] = carry[-1]
        for j in range(U2):
            t = 2 + U2 * i + j
            lastj = j == U2 - 1
            pend = block(t, pend, t + 1, OPGL if lastj else OPG, lastj,
                         fk=None if NOF else (1 + 3 * (U2 * i + j), 1 if lastj else 0))
        for j in range(U2):
            o_start(2 + U2 * i + j - 1)
        return tuple(m for ms in pend for m in ms) + (yacc[0],)
    carry = lax.fori_loop(0, (NB - 4) // U2, p2, tuple(m for ms in pend for m in ms) + (y0,))
    pend = [list(carry[4 * n:4 * n + 4]) for n in range(LA)]
    yacc[0] = carry[-1]
    pend = block(NB - 2, pend, NB - 1, OPG, fk=(37, 0))
    block(NB - 1, pend, None, OPGT, fk=(40, 1))
    o_start(NB - 3)
    o_start(NB - 2)
    ylast = yacc[0]
    if SPLIT:
        out_proj_part(NB - 1, 3, True)
    else:
        out_proj(NB - 1)

    y = _rnd(jnp.sum(ylast, axis=0, keepdims=True))
    rs = _rnd(jax.nn.sigmoid(jnp.full((1, D), rmax, F32)))
    y = _rnd(y * rs)
    o_s[pl.ds(base, 16), :] = (res_s[pl.ds(base, 16), :] + jnp.where(rowsel, y, 0.0)).astype(BF)
    o_copy(NB - 1).start()

    @pl.when(bstar != NB - 1)
    def _():
        o_copy(bstar).start()
    pltpu.make_async_copy(o_s, o_hbm, sem_o).wait()


@jax.jit
def pallas_parallel_sum__sliding_block__moe_arch_mod__prompt_kernel(
    A_x, A_wqkv, A_wo, B_x, B_w_r, B_w_gate, B_w_up, B_w_down,
):
    del B_x
    hbm = pl.BlockSpec(memory_space=pltpu.HBM)
    out = pl.pallas_call(
        kernel,
        out_shape=jax.ShapeDtypeStruct((S, D), BF),
        in_specs=[hbm] * 7,
        out_specs=hbm,
        scratch_shapes=[
            pltpu.VMEM((S, D), BF),
            pltpu.VMEM((3, D, D), BF),
            pltpu.VMEM((D, D), BF),
            pltpu.VMEM((D,), BF),
            pltpu.VMEM((F, D), BF),
            pltpu.VMEM((F, D), BF),
            pltpu.VMEM((F, D), BF),
            pltpu.VMEM((4, 2, HB, D), I32),
            pltpu.VMEM((S, D), F32),
            pltpu.VMEM((H, (NB + 1) * HB, 128), I32),
            pltpu.VMEM((NB, D // 2, BQ), I32),
            pltpu.VMEM((NB, D // 2, BQ), I32),
            pltpu.VMEM((776, D), I32),
            pltpu.VMEM((D // 2, D), I32),
            pltpu.VMEM((2, D // 2, BQ), I32),
            pltpu.VMEM((NB, 8, BQ), F32),
            pltpu.VMEM((NBUF, 4, 256, 128), F32),
            pltpu.VMEM((S, D), BF),
            pltpu.VMEM((8, D), F32),
            pltpu.SemaphoreType.DMA((NB,)),
            pltpu.SemaphoreType.DMA((8,)),
            pltpu.SemaphoreType.DMA(()),
        ],
        compiler_params=pltpu.CompilerParams(vmem_limit_bytes=100 * 2**20),
    )(A_x.reshape(S, D), A_wqkv, A_wo, B_w_r, B_w_gate.T, B_w_up.T, B_w_down)
    return out.reshape(1, S, D)
```

```python
import math

import jax
import jax.numpy as jnp
from jax import lax
import jax.experimental.pallas as pl
import jax.experimental.pallas.tpu as pltpu

S, D, H, DH, W, F = 2048, 512, 32, 16, 256, 1376
BQ = 128
HB = BQ // 2
NB = S // BQ
BF = jnp.bfloat16
F32 = jnp.float32
I32 = jnp.int32
NT = (((1,), (1,)), ((), ()))
TN = (((0,), (0,)), ((), ()))
QSCALE = (DH ** -0.5) * math.log2(math.e)
NEG = -1e30
FP = 32
LA = 3
NBUF = 4
UNROLL = 4


def _pack(v):
    return pltpu.bitcast(v.astype(BF), I32)


def _pack_pi(v):
    n = v.shape[0] // 16
    v4 = v.reshape(n, 2, 8, v.shape[1])
    return pltpu.pack_elementwise([v4[:, 0], v4[:, 1]], packed_dtype=BF).reshape(8 * n, v.shape[1])


def _unpack(v):
    return pltpu.bitcast(v, BF)


def _rnd(v):
    return v.astype(BF).astype(F32)


def _layernorm(xf):
    mean = jnp.mean(xf, axis=-1, keepdims=True)
    c = xf - mean
    var = jnp.mean(c * c, axis=-1, keepdims=True)
    d = _rnd(xf - _rnd(mean))
    s = _rnd(jnp.sqrt(_rnd(_rnd(var) + 1e-5)))
    return d / s


def _kernel(x_hbm, wqkv_hbm, wo_hbm, wr_hbm, wgt_hbm, wut_hbm, wd_hbm, o_hbm,
            x_s, wqkv_s, wo_in, wr_s, wgt_s, wut_s, wd_s,
            xn_s, res_s, ks_s, v_s, q_s, wt_s, wo_s, ot_s, r_s, s_s, o_s, xr_s,
            sem_x, sem_w, sem_o):
    def x_copy(b):
        return pltpu.make_async_copy(x_hbm.at[b * BQ:(b + 1) * BQ, :], x_s.at[b * BQ:(b + 1) * BQ, :], sem_x.at[b])

    def w_copy(i):
        return pltpu.make_async_copy(wqkv_hbm.at[:, i * D:(i + 1) * D], wqkv_s.at[i], sem_w.at[i])

    c_wr = pltpu.make_async_copy(wr_hbm, wr_s, sem_w.at[3])
    c_wo = pltpu.make_async_copy(wo_hbm, wo_in, sem_w.at[4])
    c_wg = pltpu.make_async_copy(wgt_hbm, wgt_s, sem_w.at[5])
    c_wu = pltpu.make_async_copy(wut_hbm, wut_s, sem_w.at[6])
    c_wd = pltpu.make_async_copy(wd_hbm, wd_s, sem_w.at[7])

    for c in (c_wr, x_copy(0), x_copy(1), w_copy(1), w_copy(0), x_copy(2), w_copy(2), x_copy(3)):
        c.start()

    lane8 = lax.broadcasted_iota(I32, (8, 128), 1)
    zero8 = jnp.zeros((8, 128), I32)
    jbit = [((lane8 >> 4) & (1 << k)) != 0 for k in range(3)]

    def ln_rows(b, slot, r0, n):
        t0 = b * BQ + r0
        xf = x_s[pl.ds(t0, n), :].astype(F32)
        xn = _rnd(_layernorm(xf))
        xn_s[slot, 0, r0 // 2:(r0 + n) // 2, :] = _pack(xn)
        xn_s[slot, 1, r0 // 2:(r0 + n) // 2, :] = _pack_pi(xn)
        res_s[pl.ds(t0, n), :] = xf + xn
        return pltpu.bitcast(xn[n - 8:n, 384:512], I32)

    def proj(b, slot, kind, c, z=None):
        r0 = kind * 256 + c * 128
        r1 = r0 + 128 + (8 if (kind == 2 and c == 1) else 0)
        xn = _unpack(xn_s[slot, 1 if kind == 2 else 0])
        w = wt_s[r0:r1, :]
        if z is not None:
            w = jnp.concatenate([jnp.concatenate([w[0:8, 0:128] | z, w[0:8, 128:]], axis=1), w[8:]], axis=0)
        o = lax.dot_general(_unpack(w), xn, NT, preferred_element_type=F32)
        if kind == 0:
            q_s[b, c * 128:(c + 1) * 128, :] = _pack_pi(o * QSCALE)
        elif kind == 1:
            return _pack_pi(o)
        else:
            v_s[b, c * 128:(c + 1) * 128, :] = _pack(o[0:256])
            if c == 1:
                r_s[b] = o[256:264]

    def build_ks(b, pairs, slabs, t_prev, t_cur):
        for p in pairs:
            hs = (2 * p, 2 * p + 1)
            if slabs is not None:
                rows = [slabs[h // 16][(h % 16) * 8:(h % 16 + 1) * 8] for h in hs for _ in range(8)]
                tt = pltpu.bitcast(_unpack(jnp.concatenate(rows, axis=0)).T, I32)
            for n, h in enumerate(hs):
                if slabs is not None:
                    t_cur[h] = tt[:, n * 128:(n + 1) * 128]
                g = [None if t_prev is None else t_prev[h][8 * i:8 * i + 8] for i in range(8)] + \
                    [None if slabs is None else t_cur[h][8 * i:8 * i + 8] for i in range(7)]
                for k in (2, 1, 0):
                    sh = 1 << k
                    nxt = []
                    for i in range(len(g) - sh):
                        lo, hi = g[i], g[i + sh]
                        if lo is None and hi is None:
                            nxt.append(None)
                        else:
                            nxt.append(jnp.where(jbit[k], zero8 if hi is None else hi, zero8 if lo is None else lo))
                    g = nxt
                ks_s[h, b * HB:(b + 1) * HB, :] = jnp.concatenate([zero8 if x is None else x for x in g], axis=0)

    def t_weight(i, kind):
        wt_s[kind * 256:(kind + 1) * 256, :] = pltpu.bitcast(wqkv_s[i].T, I32)

    t_even, t_odd = {}, {}
    x_copy(0).wait()
    x_copy(1).wait()
    ln_rows(0, 2, 0, BQ)
    ln_rows(1, 3, 0, BQ)
    w_copy(1).wait()
    c_wr.wait()
    for b in range(4, NB):
        x_copy(b).start()
    c_wo.start()
    c_wg.start()
    c_wu.start()
    c_wd.start()
    t_weight(1, 1)
    wt_s[768:776, :] = pltpu.bitcast(jnp.broadcast_to(wr_s[...].reshape(1, D), (16, D)), I32)
    kt = [[proj(b, 2 + b, 1, c) for c in range(2)] for b in (0, 1)]
    w_copy(0).wait()
    t_weight(0, 0)
    xb = pltpu.bitcast(x_s[0:16, 0:128], I32)
    zvec = (xb * xb + xb) & 1

    def pro_builds(n):
        build_ks(0, range(2 * n, 2 * n + 2), kt[0], None, t_even)
        build_ks(1, range(2 * n, 2 * n + 2), kt[1], t_even, t_odd)

    for b in (0, 1):
        for c in range(2):
            pro_builds(2 * b + c)
            proj(b, 2 + b, 0, c)
    w_copy(2).wait()
    x_copy(2).wait()
    t_weight(2, 2)
    lnz = [None, ln_rows(2, 0, 0, 64), ln_rows(2, 0, 64, 32), ln_rows(2, 0, 96, 32)]
    for b in (0, 1):
        for c in range(2):
            pro_builds(4 + 2 * b + c)
            proj(b, 2 + b, 2, c, None if lnz[2 * b + c] is None else lnz[2 * b + c] & zvec)

    def proj_block(b, src, dst, t_prev, t_cur):
        cur = []
        n = 0
        for kind in (1, 0, 2):
            for c in range(2):
                if 1 <= n <= 4 and dst is not None:
                    ln_rows(b + 1, dst, (n - 1) * 32, 32)
                if n in (2, 4):
                    build_ks(b, range(4 * n - 8, 4 * n), cur, t_prev, t_cur)
                o = proj(b, src, kind, c)
                if kind == 1:
                    cur.append(o)
                n += 1

    for b in range(2, NB):
        if b == 2:
            for bb in range(3, 10):
                x_copy(bb).wait()
        if b == 9:
            for bb in range(10, NB):
                x_copy(bb).wait()
            c_wo.wait()
            c_wg.wait()
            c_wu.wait()
            c_wd.wait()
        j = b % 2
        proj_block(b, j, 1 - j if b + 1 < NB else None, (t_odd, t_even)[j], (t_even, t_odd)[j])

    wo_s[...] = _pack_pi(wo_in[...].astype(F32))
    r = _rnd(r_s[...])[:, 0, :]
    rmax = jnp.max(r)
    ln = lax.broadcasted_iota(I32, (NB, BQ), 1)
    pos = lax.broadcasted_iota(I32, (NB, BQ), 0) * BQ + (ln & -16) + ((ln & 15) >> 1) + 8 * (ln & 1)
    idx = jnp.min(jnp.where(r == rmax, pos, S))
    idx = jnp.minimum(idx, S - 1)
    bstar = idx // BQ
    base = pl.multiple_of((idx // 16) * 16, 16)
    rowsel = lax.broadcasted_iota(I32, (16, 1), 0) == (idx - base)
    slab = _rnd(_layernorm(x_s[pl.ds(base, 16), :].astype(F32)))
    xr_s[...] = jnp.broadcast_to(jnp.sum(jnp.where(rowsel, slab, 0.0), axis=0, keepdims=True), (8, D))
    dzero = jnp.minimum(idx, 0)

    yacc = [None]

    def ffn_piece(k, rel=None):
        f0 = k * FP if isinstance(k, int) else pl.multiple_of(k * FP, FP)
        xr = xr_s[...]
        if rel is not None:
            xr = pltpu.bitcast(pltpu.bitcast(xr, I32) | jnp.concatenate([rel] * 4, axis=1), F32)
        xr = xr[0:1, :]
        g = _rnd(jnp.sum(wgt_s[pl.ds(f0, FP), :].astype(F32) * xr, axis=1, keepdims=True))
        u = _rnd(jnp.sum(wut_s[pl.ds(f0, FP), :].astype(F32) * xr, axis=1, keepdims=True))
        h = _rnd(_rnd(g * jax.nn.sigmoid(g)) * u)
        yp = wd_s[pl.ds(f0, FP), :].astype(F32) * h
        yp = jnp.sum(yp.reshape(FP // 8, 8, D), axis=0)
        yacc[0] = yacc[0] + yp
        return pltpu.bitcast(yp[:, 0:128], I32)

    def ffn_group(k0, rel):
        w = None
        for p in range(3):
            v = ffn_piece(k0 + p, rel)
            w = v if w is None else w | v
        return w & dzero

    maskd = lax.broadcasted_iota(I32, (16, 128), 0) <= (lax.broadcasted_iota(I32, (16, 128), 1) & 15)
    lane16 = lax.broadcasted_iota(I32, (16, 128), 1)
    ones8 = jnp.full((8, 128), 0x3F803F80, I32)
    jmask = [(lane8 >> 4) == j for j in range(8)]

    def first_group(t):
        return max(9 - 8 * t, 0) if isinstance(t, int) else 0

    def qk(t, G, par, z=None):
        i0 = first_group(t)
        ms = []
        for jh in range(4):
            h = 4 * G + jh
            row0 = (t - 1) * HB + 8 * i0
            if not isinstance(t, int):
                row0 = pl.multiple_of(row0, HB)
            kall = ks_s[h, pl.ds(row0, 8 * (17 - i0)), :]
            if i0 == 0:
                kall = jnp.concatenate([kall[0:8], kall[128:136], kall[8:128]], axis=0)
            if z is not None and jh == 0:
                kall = jnp.concatenate([kall[0:8] | z, kall[8:]], axis=0)
            qh = q_s[t, h * 8:(h + 1) * 8, :]
            qm = jnp.concatenate([jnp.where(jmask[j], qh, 0) for j in range(8)], axis=0)
            st = jnp.dot(_unpack(kall), _unpack(qm), preferred_element_type=F32)
            if i0 == 0:
                comb = jnp.where(maskd, st[16:32], st[0:16])
                mid = st[32:272]
            else:
                nm = 16 - i0
                comb = jnp.where(maskd, st[16 * nm:], NEG)
                mid = jnp.concatenate([
                    jnp.where(lane16 >= 16 * (16 - 8 * t - i), st[16 * (i - i0):16 * (i - i0 + 1)], NEG)
                    for i in range(i0, 16)], axis=0)
            nm = mid.shape[0]
            m = jnp.maximum(jnp.max(comb.reshape(2, 8, 128), axis=0), jnp.max(mid.reshape(nm // 8, 8, 128), axis=0))
            s_s[par, jh, 0:16, :] = comb
            s_s[par, jh, 16:16 + nm, :] = mid
            ms.append(jnp.max(m, axis=0, keepdims=True))
        return ms

    def unskew(plist):
        cur = plist
        for k in range(3):
            sh = 1 << k
            nxt = []
            for i in range(len(cur) + sh):
                a = cur[i - sh] if 0 <= i - sh < len(cur) else None
                b = cur[i] if i < len(cur) else None
                if a is None and b is None:
                    nxt.append(None)
                else:
                    nxt.append(jnp.where(jbit[k], zero8 if a is None else a, zero8 if b is None else b))
            cur = nxt
        return cur

    def softmax(t, G, par, ms):
        i0 = first_group(t)
        nm = 16 * (16 - max(i0, 1))
        us = []
        for jh in range(4):
            m = ms[jh]
            pc = jnp.exp2(s_s[par, jh, 0:16, :] - m)
            pm = _pack_pi(jnp.exp2(s_s[par, jh, 16:16 + nm, :] - m))
            plist = [None] * 17
            first_mid = 16 - nm // 16
            for i in range(nm // 16):
                plist[first_mid + i] = pm[8 * i:8 * i + 8]
            if i0 == 0:
                plist[0] = _pack_pi(jnp.where(maskd, 0.0, pc))
                plist[16] = _pack_pi(jnp.where(maskd, pc, 0.0))
            else:
                plist[16] = _pack_pi(pc)
            us.append(unskew(plist))
        return us

    def pv(t, G, us):
        for jh in range(4):
            h = 4 * G + jh
            u = us[jh]
            ov = None
            for T in range(3):
                if isinstance(t, int) and t - 2 + T < 0:
                    continue
                tile = jnp.concatenate([zero8 if x is None else x for x in u[8 * T:8 * T + 8]], axis=0)
                vh = v_s[t - 2 + T, h * 8:(h + 1) * 8, :]
                vv = _unpack(jnp.concatenate([vh, ones8], axis=0))
                part = jnp.dot(vv, _unpack(tile), preferred_element_type=F32)
                ov = part if ov is None else ov + part
            l = ov[16:24]
            rc = pl.reciprocal(l, approx=True)
            rc = rc * (2.0 - l * rc)
            ot_s[t % 2, h * 8:(h + 1) * 8, :] = _pack_pi((ov[0:16].reshape(2, 8, 128) * rc).reshape(16, 128))

    def out_proj(b):
        t0 = b * BQ if isinstance(b, int) else pl.multiple_of(b * BQ, BQ)
        a = lax.dot_general(_unpack(ot_s[b % 2]), _unpack(wo_s[...]), TN, preferred_element_type=F32)
        o32 = res_s[pl.ds(t0, BQ), :] + a
        res_s[pl.ds(t0, BQ), :] = o32
        o_s[pl.ds(t0, BQ), :] = o32.astype(BF)
        return pltpu.bitcast(a[0:8, 0:128], I32)

    def out_proj_part(b, g, last=False):
        a = lax.dot_general(_unpack(ot_s[b % 2, g * 64:(g + 1) * 64, :]), _unpack(wo_s[g * 64:(g + 1) * 64, :]),
                            TN, preferred_element_type=F32)
        o32 = res_s[b * BQ:(b + 1) * BQ, :] + a
        res_s[b * BQ:(b + 1) * BQ, :] = o32
        if last:
            o_s[b * BQ:(b + 1) * BQ, :] = o32.astype(BF)

    def o_copy(b):
        t0 = b * BQ if isinstance(b, int) else pl.multiple_of(b * BQ, BQ)
        return pltpu.make_async_copy(o_s.at[pl.ds(t0, BQ), :], o_hbm.at[pl.ds(t0, BQ), :], sem_o)

    def o_start(b):
        @pl.when(b != bstar)
        def _():
            o_copy(b).start()

    def block(t, pend, nt, prev_out, last=False, fk=None):
        rel = None
        pend = list(pend)
        for G in range(8):
            def next_qk():
                n = G + LA
                if n < 8:
                    z = None
                    if fk is not None and fk[1] == 0 and G == 4:
                        z = ffn_group(fk[0], rel)
                    return qk(t, n, n % NBUF, z)
                return None if nt is None else qk(nt, n - 8, n % NBUF)
            late = last and G == 7
            if isinstance(t, int) and t < 2:
                build_ks(NB, [8 * t + G], None, t_odd, None)
            us = softmax(t, G, G % NBUF, pend.pop(0))
            if not late:
                pend.append(next_qk())
            if G == prev_out:
                a0 = out_proj(t - 1)
                if fk is not None and fk[1] == 1:
                    ffn_group(fk[0], a0 & dzero)
                if fk is not None and fk[1] == 0:
                    rel = a0 & dzero
            pv(t, G, us)
            if late:
                pend.append(next_qk())
            if isinstance(t, int) and t == NB - 1 and G in (3, 5, 7):
                out_proj_part(t, (G - 3) // 2)
        return pend

    pend = [qk(0, n, n % NBUF) for n in range(LA)]
    pend = block(0, pend, 1, None)
    yacc[0] = jnp.zeros((8, D), F32)
    ffn_piece(0)
    y0 = yacc[0]
    pend = block(1, pend, 2, 7, True)
    o_start(0)

    def attend(i, carry):
        pend = [list(carry[4 * n:4 * n + 4]) for n in range(LA)]
        yacc[0] = carry[-1]
        for j in range(UNROLL):
            t = 2 + UNROLL * i + j
            lastj = j == UNROLL - 1
            pend = block(t, pend, t + 1, 4 if lastj else 3, lastj, fk=(1 + 3 * (UNROLL * i + j), 1 if lastj else 0))
        for j in range(UNROLL):
            o_start(2 + UNROLL * i + j - 1)
        return tuple(m for ms in pend for m in ms) + (yacc[0],)

    carry = lax.fori_loop(0, (NB - 4) // UNROLL, attend, tuple(m for ms in pend for m in ms) + (y0,))
    pend = [list(carry[4 * n:4 * n + 4]) for n in range(LA)]
    yacc[0] = carry[-1]
    pend = block(NB - 2, pend, NB - 1, 3, fk=(37, 0))
    block(NB - 1, pend, None, 4, fk=(40, 1))
    o_start(NB - 3)
    o_start(NB - 2)
    ylast = yacc[0]
    out_proj_part(NB - 1, 3, True)

    y = _rnd(jnp.sum(ylast, axis=0, keepdims=True))
    rs = _rnd(jax.nn.sigmoid(jnp.full((1, D), rmax, F32)))
    y = _rnd(y * rs)
    o_s[pl.ds(base, 16), :] = (res_s[pl.ds(base, 16), :] + jnp.where(rowsel, y, 0.0)).astype(BF)
    o_copy(NB - 1).start()

    @pl.when(bstar != NB - 1)
    def _():
        o_copy(bstar).start()
    pltpu.make_async_copy(o_s, o_hbm, sem_o).wait()


@jax.jit
def pallas_parallel_sum__sliding_block__moe_arch_mod__prompt_kernel(
    A_x, A_wqkv, A_wo, B_x, B_w_r, B_w_gate, B_w_up, B_w_down,
):
    del B_x
    hbm = pl.BlockSpec(memory_space=pltpu.HBM)
    out = pl.pallas_call(
        _kernel,
        out_shape=jax.ShapeDtypeStruct((S, D), BF),
        in_specs=[hbm] * 7,
        out_specs=hbm,
        scratch_shapes=[
            pltpu.VMEM((S, D), BF),
            pltpu.VMEM((3, D, D), BF),
            pltpu.VMEM((D, D), BF),
            pltpu.VMEM((D,), BF),
            pltpu.VMEM((F, D), BF),
            pltpu.VMEM((F, D), BF),
            pltpu.VMEM((F, D), BF),
            pltpu.VMEM((4, 2, HB, D), I32),
            pltpu.VMEM((S, D), F32),
            pltpu.VMEM((H, (NB + 1) * HB, 128), I32),
            pltpu.VMEM((NB, D // 2, BQ), I32),
            pltpu.VMEM((NB, D // 2, BQ), I32),
            pltpu.VMEM((776, D), I32),
            pltpu.VMEM((D // 2, D), I32),
            pltpu.VMEM((2, D // 2, BQ), I32),
            pltpu.VMEM((NB, 8, BQ), F32),
            pltpu.VMEM((NBUF, 4, 256, 128), F32),
            pltpu.VMEM((S, D), BF),
            pltpu.VMEM((8, D), F32),
            pltpu.SemaphoreType.DMA((NB,)),
            pltpu.SemaphoreType.DMA((8,)),
            pltpu.SemaphoreType.DMA(()),
        ],
        compiler_params=pltpu.CompilerParams(vmem_limit_bytes=100 * 2**20),
    )(A_x.reshape(S, D), A_wqkv, A_wo, B_w_r, B_w_gate.T, B_w_up.T, B_w_down)
    return out.reshape(1, S, D)
```
